```python
import os as _os
_os.environ.setdefault("JAX_PLATFORMS", "cpu")
import jax
import jax.numpy as jnp

def _softmax(x, axis=-1):
    return jax.nn.softmax(x, axis=axis)
def _gelu(x):
    return jax.nn.gelu(x, approximate=True)
def _silu(x):
    return jax.nn.silu(x)
def _sigmoid(x):
    return jax.nn.sigmoid(x)
def _layernorm(x, axis=-1, eps=1e-5):
    m = jnp.mean(x, axis=axis, keepdims=True)
    v = jnp.var(x, axis=axis, keepdims=True)
    return (x - m) / jnp.sqrt(v + eps)
def _scatter_add(tgt, idx, src, axis=0):
    return tgt.at[idx].add(src)
def _segment_sum(src, seg, n):
    return jax.ops.segment_sum(src, seg, n)
class _Rng:
    def __init__(self, key):
        self._k = key
    def _next(self):
        self._k, sub = jax.random.split(self._k)
        return sub
    def normal(self, shape):
        return jax.random.normal(self._next(), shape, dtype=jnp.bfloat16)
    def randint(self, lo, hi, shape):
        return jax.random.randint(self._next(), shape, lo, hi, dtype=jnp.int32)
    def uniform(self, shape, lo=0.0, hi=1.0):
        return jax.random.uniform(self._next(), shape, jnp.bfloat16, lo, hi)
    def permutation(self, n):
        return jax.random.permutation(self._next(), n)


kernel_name = 'concat_heads__ssm_conv_s4__linear_attn_block__prompt'

def setup_inputs():
    _rng = _Rng(jax.random.key(int.from_bytes(__import__("os").urandom(4), "little")))
    _w = (lambda a: (lambda t: t.astype(jnp.bfloat16) if jnp.issubdtype(t.dtype, jnp.floating) else t)(jnp.asarray(a)))
    def _A_setup():
        B, L, D, N = 1, 2048, 512, 128
        A_re = -jnp.exp((lambda *s: _rng.normal(s) * 0.1)(D, N))
        A_im = jnp.pi * (lambda *s: _rng.normal(s) * 0.1)(D, N)
        B_re = (lambda *s: _rng.normal(s) * 0.1)(D, N)
        B_im = (lambda *s: _rng.normal(s) * 0.1)(D, N)
        C_re = (lambda *s: _rng.normal(s) * 0.1)(D, N)
        C_im = (lambda *s: _rng.normal(s) * 0.1)(D, N)
        log_dt = (lambda *s: _rng.normal(s) * 0.1)(D) * 0.5 - 4.0
        Dskip = (lambda *s: _rng.normal(s) * 0.05)(D)
        return {
            "u": _w((lambda *s: _rng.normal(s) * 0.05)(B, L, D)),
            "A_re": _w(A_re),
            "A_im": _w(A_im),
            "B_re": _w(B_re),
            "B_im": _w(B_im),
            "C_re": _w(C_re),
            "C_im": _w(C_im),
            "log_dt": _w(log_dt),
            "Dskip": _w(Dskip),
        }
    _A_in = _A_setup()

    def _B_setup():
        B, S, D = 1, 2048, 512
        return {
            "x": _w((lambda *s: _rng.normal(s) * 0.05)(B, S, D)),
            "wqkv": _w((lambda *s: _rng.normal(s) * 0.4)(D, 3 * D)),
            "wo": _w((lambda *s: _rng.normal(s) * 0.05)(D, D)),
        }
    _B_in = _B_setup()

    return {
        "A_u": _A_in["u"],
        "A_A_re": _A_in["A_re"],
        "A_A_im": _A_in["A_im"],
        "A_B_re": _A_in["B_re"],
        "A_B_im": _A_in["B_im"],
        "A_C_re": _A_in["C_re"],
        "A_C_im": _A_in["C_im"],
        "A_log_dt": _A_in["log_dt"],
        "A_Dskip": _A_in["Dskip"],
        "B_x": _B_in["x"],
        "B_wqkv": _B_in["wqkv"],
        "B_wo": _B_in["wo"],
    }

def reference(A_u, A_A_re, A_A_im, A_B_re, A_B_im, A_C_re, A_C_im, A_log_dt, A_Dskip, B_x, B_wqkv, B_wo):
    def _A_ref(u, A_re, A_im, B_re, B_im, C_re, C_im, log_dt, Dskip):
        Bsz, L, D = u.shape
        dt = jnp.exp(log_dt)[:, None]
        A = A_re + 1j * A_im
        Bc = B_re + 1j * B_im
        Cc = C_re + 1j * C_im
        logdA = dt * A
        dB = dt * Bc
        l = (lambda x, dt: x.astype(dt))(jnp.arange(L), A_re.dtype)
        P = jnp.exp(logdA[:, :, None] * l[None, None, :])
        K = jnp.einsum("dn,dnl,dn->dl", Cc, P, dB).real
        L2 = 2 * L
        Kp = jnp.pad(K, ((0, 0), (0, L)))
        up = (lambda x, *d: x.transpose(*d))(u, 0, 2, 1)
        up = jnp.pad(up, ((0, 0), (0, 0), (0, L)))
        Kf = (lambda x, axes=(-2,-1): jnp.fft.rfft2(x.astype(jnp.float32), axes=axes))(Kp[:, None, :], axes=(-2, -1))
        Uf = (lambda x, axes=(-2,-1): jnp.fft.rfft2(x.astype(jnp.float32), axes=axes))(up[:, :, None, :], axes=(-2, -1))
        Yf = Uf * Kf[None, :, :, :]
        y = (lambda x, s, axes=(-2,-1): jnp.fft.irfft2(x, s=s, axes=axes).astype(jnp.bfloat16))(Yf, (1, L2), axes=(-2, -1))[:, :, 0, :L]
        y = (lambda x, *d: x.transpose(*d))(y, 0, 2, 1) + u * Dskip[None, None, :]
        return y

    def _B_ref(x, wqkv, wo):
        B, S, D = x.shape
        H = 32; Dh = D // H
        qkv = (lambda x, *d: x.transpose(*d))((x @ wqkv).reshape(B, S, 3, H, Dh), 2, 0, 3, 1, 4)
        q, k, v = qkv[0], qkv[1], qkv[2]
        phi = lambda t: jnp.where(t > 0, t + 1, jnp.exp(t)) + 1e-6
        pq, pk = phi(q), phi(k)
        kv = jnp.einsum("bhsd,bhse->bhde", pk, v)
        z = jnp.einsum("bhsd->bhd", pk)
        num = jnp.einsum("bhqd,bhde->bhqe", pq, kv)
        den = jnp.einsum("bhqd,bhd->bhq", pq, z)[..., None] + 1e-6
        o = num / den
        return (lambda x, *d: x.transpose(*d))(o, 0, 2, 1, 3).reshape(B, S, D) @ wo

    a = _A_ref(A_u, A_A_re, A_A_im, A_B_re, A_B_im, A_C_re, A_C_im, A_log_dt, A_Dskip)
    b = _B_ref(B_x, B_wqkv, B_wo)
    return jnp.concatenate([a, b], axis=-1)
```

```python
import functools

import numpy as np
import jax
import jax.numpy as jnp
from jax import lax
import jax.experimental.pallas as pl
import jax.experimental.pallas.tpu as pltpu

L = 2048
D = 512
NS = 128
C = 128
NCH = L // C
H = 32
DH = D // H

F32 = jnp.float32
BF16 = jnp.bfloat16


def _row_exponents():
    rows = []
    for i in range(NCH):
        rhos = range(8) if i < 2 else (0, 2, 4, 6) if i < 4 else (0, 4) if i < 8 else (0,)
        rows += [C * i + r for r in rhos]
    return rows + [2048]


ROW_E = _row_exponents()
NROWS = len(ROW_E)
SLOTS = [(a // 8, a % 8, a) for a in range(40)] + [
    (5, 0, ROW_E.index(512)), (5, 1, ROW_E.index(1024)), (5, 2, 40)]


@functools.lru_cache(maxsize=None)
def _constants():
    bf = jnp.bfloat16
    rl = np.arange(L).astype(np.float32).astype(bf).astype(np.int64)
    kperm = np.concatenate([np.arange(0, C, 2), np.arange(1, C, 2)])

    def w(j):
        return np.exp(-1j * np.pi * (2 * kperm + 1) * j / 256.0)

    own_tile = {}
    for (t, s, a) in SLOTS[:40]:
        own_tile[ROW_E[a] // C] = t
    pairs = {}
    for al in range(NCH):
        for j in range(C):
            v = int(rl[C * al + j])
            cand = [(t, s) for (t, s, a) in SLOTS
                    if v >= ROW_E[a] and (v - ROW_E[a]) % 8 == 0 and (v - ROW_E[a]) // 8 < 16]
            e_of = {(t, s): ROW_E[a] for (t, s, a) in SLOTS}
            same = [c for c in cand if c[0] == own_tile[al]]
            t, s = same[0] if same else [c for c in cand if c[0] == 5][0]
            b = (v - e_of[(t, s)]) // 8
            m = pairs.setdefault((al, t), np.zeros((C, C), np.complex128))
            m[:, 8 * ((b + 1) % 16) + s] += w(j)
    keys = sorted(pairs.keys())
    fsel = np.stack([np.concatenate([pairs[k].real, pairs[k].imag], 0) for k in keys])
    ff = np.stack([w(j) for j in range(C)], 1)
    ffwd = np.concatenate([ff.real, ff.imag], 0)
    tau = np.arange(C)
    ang = 2 * np.pi * (kperm[None, :] + 0.5) * (C + tau[:, None]) / 256.0
    finv = np.concatenate([np.cos(ang), -np.sin(ang)], 1) * (2.0 / 256.0)
    hid = np.arange(128) // DH
    bmask = (hid[:, None] == hid[None, :]).astype(np.float32)
    return (tuple(keys), fsel.astype(bf), ffwd.astype(bf), finv.astype(bf), bmask.astype(bf))


def _cmul(ar, ai, br, bi):
    return ar * br - ai * bi, ar * bi + ai * br


def _nt(a, b):
    return lax.dot_general(a, b, (((1,), (1,)), ((), ())), preferred_element_type=F32)


def _tn(a, b):
    return lax.dot_general(a, b, (((0,), (0,)), ((), ())), preferred_element_type=F32)


def _nn(a, b):
    return jnp.dot(a, b, preferred_element_type=F32)


def _phi(t):
    return jnp.where(t > 0, t + 1.0, jnp.exp(t)) + 1e-6


def _rev8(x):
    r = x.shape[0]
    sub = lax.broadcasted_iota(jnp.int32, x.shape, 0) % 8
    x3 = x
    for bit in (4, 2, 1):
        up = pltpu.roll(x3, r - bit, 0)
        dn = pltpu.roll(x3, bit, 0)
        x3 = jnp.where((sub & bit) == 0, up, dn)
    return x3


GPI = 4
RB = 8 * GPI


def _kernel(keys,
            u_hbm, are_ref, aim_ref, bre_ref, bim_ref, cre_ref, cim_ref, ldt_ref, dsk_ref,
            x_hbm, wqkv_hbm, wo_hbm, fsel_hbm, ffwd_hbm, finv_hbm, bmask_hbm,
            out_hbm,
            u_v, x_v, wqkv_v, wo_v, fsel_v, ffwd_v, finv_v, bmask_v,
            tab_v, kt_v, kp_v, kq_v, kr_v, us_v, ua_v, ub_v, yh_v,
            pk_v, v_v, m_v, z_v, oa_v, ob_v, sems, osems):
    copies = [
        pltpu.make_async_copy(x_hbm, x_v, sems.at[0]),
        pltpu.make_async_copy(wqkv_hbm, wqkv_v, sems.at[1]),
        pltpu.make_async_copy(fsel_hbm, fsel_v, sems.at[2]),
        pltpu.make_async_copy(u_hbm, u_v, sems.at[3]),
        pltpu.make_async_copy(ffwd_hbm, ffwd_v, sems.at[4]),
        pltpu.make_async_copy(finv_hbm, finv_v, sems.at[5]),
        pltpu.make_async_copy(wo_hbm, wo_v, sems.at[6]),
        pltpu.make_async_copy(bmask_hbm, bmask_v, sems.at[7]),
    ]
    for c in copies:
        c.start()

    dt_row = jnp.exp(ldt_ref[...].astype(F32)).astype(BF16).astype(F32)
    dt = jnp.transpose(jnp.broadcast_to(dt_row, (128, D)))
    lre = dt * are_ref[...].astype(F32)
    lim = dt * aim_ref[...].astype(F32)
    mag = jnp.exp(lre)
    l1r = mag * jnp.cos(lim)
    l1i = mag * jnp.sin(lim)
    dbr = dt * bre_ref[...].astype(F32)
    dbi = dt * bim_ref[...].astype(F32)
    cr, ci = _cmul(cre_ref[...].astype(F32), cim_ref[...].astype(F32), dbr, dbi)
    l2r, l2i = _cmul(l1r, l1i, l1r, l1i)
    l4r, l4i = _cmul(l2r, l2i, l2r, l2i)
    l8r, l8i = _cmul(l4r, l4i, l4r, l4i)
    tab_v[0] = l1r
    tab_v[1] = l1i
    tab_v[2] = cr
    tab_v[3] = ci
    tab_v[4] = _rev8(l8r)
    tab_v[5] = _rev8(l8i)
    tab_v[6] = l8r
    tab_v[7] = l8i

    lane = lax.broadcasted_iota(jnp.int32, (8, 128), 1)

    def kgen(it, carry):
        r0 = pl.multiple_of(it * RB, RB)
        rows = pl.ds(r0, RB)
        p1 = (tab_v[0, rows, :], tab_v[1, rows, :])
        c0 = (tab_v[2, rows, :], tab_v[3, rows, :])
        h8 = (tab_v[4, rows, :], tab_v[5, rows, :])
        p8 = (tab_v[6, rows, :], tab_v[7, rows, :])
        hs = [(jnp.ones((RB, 128), F32), jnp.zeros((RB, 128), F32)), h8]
        for b in range(2, 16):
            hs.append(_cmul(*hs[-1], *h8))
        pw = {1: p1}
        pw[2] = _cmul(*p1, *p1)
        pw[3] = _cmul(*pw[2], *p1)
        pw[4] = _cmul(*pw[2], *pw[2])
        pw[5] = _cmul(*pw[4], *p1)
        pw[6] = _cmul(*pw[4], *pw[2])
        pw[7] = _cmul(*pw[4], *pw[3])
        p16 = _cmul(*p8, *p8)
        p32 = _cmul(*p16, *p16)
        p64 = _cmul(*p32, *p32)
        p128 = _cmul(*p64, *p64)
        base = {0: c0}
        for i in range(1, 17):
            base[i] = _cmul(*base[i - 1], *p128)
        gs = []
        for e in ROW_E:
            i, rho = e // C, e % C
            gs.append(base[i] if rho == 0 else _cmul(*base[i], *pw[rho]))
        zero = jnp.zeros((8, 128), F32)
        tiles = [[] for _ in range(6)]
        for q in range(GPI):
            sl = slice(8 * q, 8 * q + 8)
            gr = jnp.concatenate([g[0][sl] for g in gs] + [zero], axis=0)
            gi = jnp.concatenate([g[1][sl] for g in gs] + [zero], axis=0)
            gm = jnp.concatenate([gr, gi], axis=1).astype(BF16)
            hr = jnp.concatenate([h[0][sl] for h in hs], axis=0)
            hi = jnp.concatenate([-h[1][sl] for h in hs], axis=0)
            hm = jnp.concatenate([hr, hi], axis=1).astype(BF16)
            o = _nt(gm, hm)
            acc = [zero] * 6
            for (t, s, a) in SLOTS:
                rolled = pltpu.roll(o[8 * a:8 * a + 8], s + 1, 1, stride=1, stride_axis=0)
                acc[t] = jnp.where(lane % 8 == s, rolled, acc[t])
            for t in range(6):
                tiles[t].append(acc[t])
        for t in range(6):
            kt_v[t, rows, :] = jnp.concatenate(tiles[t], axis=0).astype(BF16)
        return carry

    lax.fori_loop(0, D // RB, kgen, 0)

    copies[2].wait()
    for al in range(NCH):
        acc = None
        for pi, (a2, t) in enumerate(keys):
            if a2 != al:
                continue
            r = _nt(fsel_v[pi], kt_v[t])
            acc = r if acc is None else acc + r
        kr = acc[:C]
        ki = acc[C:]
        kp_v[al] = kr
        kq_v[al] = ki - kr
        kr_v[al] = kr + ki

    copies[3].wait()
    copies[4].wait()
    zprev = None
    for a in range(NCH):
        z = _nn(ffwd_v[...], u_v[C * a:C * a + C, :])
        zr, zi = z[:C], z[C:]
        sgn_i = jnp.concatenate([zi[:64], -zi[64:]], axis=0)
        sgn_r = jnp.concatenate([zr[:64], -zr[64:]], axis=0)
        if zprev is None:
            ar, ai = sgn_i, -sgn_r
        else:
            ar, ai = zprev[0] + sgn_i, zprev[1] - sgn_r
        zprev = (zr, zi)
        ua_v[a] = ar
        ub_v[a] = ai
        us_v[a] = ar + ai

    copies[0].wait()
    copies[1].wait()
    copies[6].wait()
    copies[7].wait()
    SB = 256

    def kvproj(i, carry):
        r0 = pl.multiple_of(i * SB, SB)
        xb = x_v[pl.ds(r0, SB), :]
        k = _nn(xb, wqkv_v[:, D:2 * D])
        pk_v[pl.ds(r0, SB), :] = _phi(k).astype(BF16)
        v_v[pl.ds(r0, SB), :] = _nn(xb, wqkv_v[:, 2 * D:3 * D]).astype(BF16)
        return carry

    lax.fori_loop(0, L // SB, kvproj, 0)
    z_v[...] = jnp.sum(pk_v[...].astype(F32), axis=0, keepdims=True)
    for blk in range(4):
        cs = slice(128 * blk, 128 * blk + 128)
        kv = _tn(pk_v[:, cs], v_v[:, cs]) * bmask_v[...].astype(F32)
        m_v[cs, :] = _nn(kv.astype(BF16), wo_v[cs, :]).astype(BF16)

    def prod(col, carry):
        kb = col // 4
        dtile = col % 4
        rs = pl.ds(pl.multiple_of(kb * 8, 8), 8)
        cs = pl.ds(pl.multiple_of(dtile * 128, 128), 128)
        top = kb < 8
        for a0 in range(0, NCH, 4):
            acc = [[None] * 3 for _ in range(4)]
            for al in range(a0 + 4):
                kk = (kp_v[al, rs, cs], kq_v[al, rs, cs], kr_v[al, rs, cs])
                for o in range(4):
                    ap = a0 + o - al
                    if ap < 0:
                        continue
                    uu = (us_v[ap, rs, cs], ua_v[ap, rs, cs], ub_v[ap, rs, cs])
                    for w in range(3):
                        t = kk[w] * uu[w]
                        acc[o][w] = t if acc[o][w] is None else acc[o][w] + t
            for o in range(4):
                yh_v[a0 + o, rs, cs] = acc[o][0] - acc[o][2]
                yh_v[a0 + o, pl.ds(pl.multiple_of(kb * 8 + C, 8), 8), cs] = acc[o][0] + acc[o][1]
        return carry

    lax.fori_loop(0, 64, prod, 0)

    copies[5].wait()
    dsk = dsk_ref[...].astype(F32)
    zrow = z_v[...]
    for a in range(NCH):
        rs = slice(C * a, C * a + C)
        y = _nn(finv_v[...], yh_v[a].astype(BF16))
        ya = y.astype(BF16).astype(F32) + (u_v[rs, :].astype(F32) * dsk).astype(BF16).astype(F32)
        oa_v[rs, :] = ya.astype(BF16)
        pltpu.make_async_copy(oa_v.at[rs, :], out_hbm.at[rs, 0:D], osems.at[0, a]).start()
        pq = _phi(_nn(x_v[rs, :], wqkv_v[:, 0:D]))
        pz = (pq * zrow).astype(BF16)
        den = jnp.concatenate(
            [_nn(pz[:, 128 * b:128 * b + 128], bmask_v[...]) for b in range(4)], axis=1) + 1e-6
        o = (pq / den).astype(BF16)
        ob_v[rs, :] = _nn(o, m_v[...]).astype(BF16)
        pltpu.make_async_copy(ob_v.at[rs, :], out_hbm.at[rs, D:2 * D], osems.at[1, a]).start()
    for a in range(NCH):
        rs = slice(C * a, C * a + C)
        pltpu.make_async_copy(oa_v.at[rs, :], out_hbm.at[rs, 0:D], osems.at[0, a]).wait()
        pltpu.make_async_copy(ob_v.at[rs, :], out_hbm.at[rs, D:2 * D], osems.at[1, a]).wait()


@jax.jit
def pallas_concat_heads__ssm_conv_s4__linear_attn_block__prompt_kernel(
    A_u: jax.Array,
    A_A_re: jax.Array,
    A_A_im: jax.Array,
    A_B_re: jax.Array,
    A_B_im: jax.Array,
    A_C_re: jax.Array,
    A_C_im: jax.Array,
    A_log_dt: jax.Array,
    A_Dskip: jax.Array,
    B_x: jax.Array,
    B_wqkv: jax.Array,
    B_wo: jax.Array,
):
    keys, fsel, ffwd, finv, bmask = _constants()
    npair = len(keys)
    any_spec = pl.BlockSpec(memory_space=pl.ANY)
    vm = pl.BlockSpec(memory_space=pltpu.VMEM)
    out = pl.pallas_call(
        functools.partial(_kernel, keys),
        out_shape=jax.ShapeDtypeStruct((L, 2 * D), BF16),
        in_specs=[any_spec] + [vm] * 8 + [any_spec] * 7,
        out_specs=any_spec,
        scratch_shapes=[
            pltpu.VMEM((L, D), BF16),
            pltpu.VMEM((L, D), BF16),
            pltpu.VMEM((D, 3 * D), BF16),
            pltpu.VMEM((D, D), BF16),
            pltpu.VMEM((npair, 256, 128), BF16),
            pltpu.VMEM((256, 128), BF16),
            pltpu.VMEM((128, 256), BF16),
            pltpu.VMEM((128, 128), BF16),
            pltpu.VMEM((8, D, 128), F32),
            pltpu.VMEM((6, D, 128), BF16),
            pltpu.VMEM((NCH, C, D), F32),
            pltpu.VMEM((NCH, C, D), F32),
            pltpu.VMEM((NCH, C, D), F32),
            pltpu.VMEM((NCH, C, D), F32),
            pltpu.VMEM((NCH, C, D), F32),
            pltpu.VMEM((NCH, C, D), F32),
            pltpu.VMEM((NCH, 2 * C, D), F32),
            pltpu.VMEM((L, D), BF16),
            pltpu.VMEM((L, D), BF16),
            pltpu.VMEM((D, D), BF16),
            pltpu.VMEM((1, D), F32),
            pltpu.VMEM((L, D), BF16),
            pltpu.VMEM((L, D), BF16),
            pltpu.SemaphoreType.DMA((8,)),
            pltpu.SemaphoreType.DMA((2, NCH)),
        ],
        compiler_params=pltpu.CompilerParams(vmem_limit_bytes=100 * 1024 * 1024),
    )(
        A_u.reshape(L, D), A_A_re, A_A_im, A_B_re, A_B_im, A_C_re, A_C_im,
        A_log_dt.reshape(1, D), A_Dskip.reshape(1, D),
        B_x.reshape(L, D), B_wqkv, B_wo,
        jnp.asarray(fsel), jnp.asarray(ffwd), jnp.asarray(finv), jnp.asarray(bmask),
    )
    return out.reshape(1, L, 2 * D)
```

```python
import functools

import numpy as np
import jax
import jax.numpy as jnp
from jax import lax
import jax.experimental.pallas as pl
import jax.experimental.pallas.tpu as pltpu

L = 2048
D = 512
NS = 128
C = 128
NCH = L // C
H = 32
DH = D // H
ND = D // 128

F32 = jnp.float32
BF16 = jnp.bfloat16
U32 = jnp.uint32


def _row_exponents():
    rows = []
    for i in range(NCH):
        rhos = range(8) if i < 2 else (0, 2, 4, 6) if i < 4 else (0, 4) if i < 8 else (0,)
        rows += [C * i + r for r in rhos]
    return rows + [2048]


ROW_E = _row_exponents()
NROWS = len(ROW_E)
GROWS = 8 * (NROWS + 1)
SLOTS = [(a // 8, a % 8, a) for a in range(40)] + [
    (5, 0, ROW_E.index(512)), (5, 1, ROW_E.index(1024)), (5, 2, 40)]


@functools.lru_cache(maxsize=None)
def _constants():
    bf = jnp.bfloat16
    rl = np.arange(L).astype(np.float32).astype(bf).astype(np.int64)
    kperm = np.concatenate([np.arange(0, C, 2), np.arange(1, C, 2)])

    def w(j):
        return np.exp(-1j * np.pi * (2 * kperm + 1) * j / 256.0)

    own_tile = {}
    for (t, s, a) in SLOTS[:40]:
        own_tile[ROW_E[a] // C] = t
    e_of = {(t, s): ROW_E[a] for (t, s, a) in SLOTS}
    pairs = {}
    for al in range(NCH):
        for j in range(C):
            v = int(rl[C * al + j])
            cand = [(t, s) for (t, s, a) in SLOTS
                    if v >= ROW_E[a] and (v - ROW_E[a]) % 8 == 0 and (v - ROW_E[a]) // 8 < 16]
            same = [c for c in cand if c[0] == own_tile[al]]
            t, s = same[0] if same else [c for c in cand if c[0] == 5][0]
            b = (v - e_of[(t, s)]) // 8
            m = pairs.setdefault((al, t), np.zeros((C, C), np.complex128))
            m[:, 8 * ((b + 1) % 16) + s] += w(j)
    keys = sorted(pairs.keys())
    fsel = np.stack([np.concatenate([pairs[k].real, pairs[k].imag], 0) for k in keys])
    ff = np.stack([w(j) for j in range(C)], 1)
    ffwd = np.concatenate([ff.real, ff.imag], 0)
    tau = np.arange(C)
    ang = 2 * np.pi * (kperm[None, :] + 0.5) * (C + tau[:, None]) / 256.0
    finv = np.stack([np.cos(ang), -np.sin(ang)], 0) * (2.0 / 256.0)
    hid = np.arange(128) // DH
    bmask = (hid[:, None] == hid[None, :]).astype(np.float32)
    tab = np.concatenate([fsel.reshape(-1, 128), ffwd, finv.reshape(-1, 128), bmask], 0)
    return tuple(keys), tab.astype(bf)


def _cmul(ar, ai, br, bi):
    return ar * br - ai * bi, ar * bi + ai * br


def _nt(a, b):
    return lax.dot_general(a, b, (((1,), (1,)), ((), ())), preferred_element_type=F32)


def _tn(a, b):
    return lax.dot_general(a, b, (((0,), (0,)), ((), ())), preferred_element_type=F32)


def _nn(a, b):
    return jnp.dot(a, b, preferred_element_type=F32)


def _phi(t):
    return jnp.where(t > 0, t + 1.0, jnp.exp(t)) + 1e-6


def _ld(ref_u32, *idx):
    *lead, (r0, n) = idx
    return pltpu.bitcast(ref_u32[(*lead, slice(r0 // 2, (r0 + n) // 2), slice(None))], BF16)


def _pk(x):
    return pltpu.bitcast(x.astype(BF16), U32)


def _rev8(x):
    sub = lax.broadcasted_iota(jnp.int32, x.shape, 0)
    for bit in (4, 2, 1):
        up = pltpu.roll(x, 8 - bit, 0)
        dn = pltpu.roll(x, bit, 0)
        x = jnp.where((sub & bit) == 0, up, dn)
    return x


GPI = 8
RB = 8 * GPI
NKI = D // RB
PR_ = 512
QR = 256
NQ = L // QR


SCHEDULE = [
    dict(wait=['p0'], jobs=[('preka', 0)]),
    dict(wait=['x0', 'wa'], jobs=[('mp', 0), ('mp', 1), ('prekb', 0)]),
    dict(wait=['wb', 'p1'], jobs=[('mk', 0), ('mp', 2), ('mp', 3), ('postp', 0), ('postp', 1), ('prek', 1)]),
    dict(wait=['x1'], jobs=[('mk', 1), ('mp', 4), ('mp', 5), ('postk', 0), ('postp', 2), ('postp', 3), ('prek', 2)]),
    dict(jobs=[('mk', 2), ('mp', 6), ('mp', 7), ('postk', 1), ('postp', 4), ('postp', 5), ('prek', 3)]),
    dict(wait=['x2'], jobs=[('mk', 3), ('mp', 8), ('mp', 9), ('postk', 2), ('postp', 6), ('postp', 7), ('prek', 4)]),
    dict(jobs=[('mk', 4), ('mp', 10), ('mp', 11), ('postk', 3), ('postp', 8), ('postp', 9), ('prek', 5)]),
    dict(wait=['x3'], jobs=[('mk', 5), ('mp', 12), ('mp', 13), ('postk', 4), ('postp', 10), ('postp', 11), ('prek', 6)]),
    dict(jobs=[('mk', 6), ('mp', 14), ('mp', 15), ('postk', 5), ('postp', 12), ('postp', 13), ('prek', 7)]),
    dict(wait=['c', 'u'], jobs=[('mk', 7), ('kh', 0), ('z', 0), ('postk', 6), ('postp', 14), ('postp', 15)]),
    dict(wait=['wq', 'wo'], jobs=[('kvm',), ('kh', 1), ('q1', 0), ('postk', 7), ('postkh', 0), ('postz', 0)]),
    dict(jobs=[('z', 1), ('kh', 2), ('q1', 1), ('v1', 0), ('postkh', 1), ('pra', 0)]),
    dict(jobs=[('z', 2), ('q2', 0), ('q1', 2), ('kh', 3), ('v1', 1), ('postz', 1), ('postkh', 2), ('prb', 0)]),
    dict(jobs=[('inv', 0), ('z', 3), ('q1', 3), ('q2', 1), ('v1', 2), ('v2', 0), ('postz', 2), ('postkh', 3), ('pra', 1)]),
    dict(jobs=[('q1', 4), ('q2', 2), ('q3', 0), ('q1', 5), ('v1', 3), ('v2', 1), ('postinv', 0), ('postz', 3), ('prb', 1)]),
    dict(jobs=[('inv', 1), ('q2', 3), ('q3', 1), ('q1', 6), ('v1', 4), ('v1', 5), ('v2', 2), ('v3', 0), ('pra', 2)]),
    dict(jobs=[('q1', 7), ('q2', 4), ('q2', 5), ('q3', 2), ('v1', 6), ('v2', 3), ('v3', 1), ('postinv', 1), ('prb', 2)]),
    dict(jobs=[('inv', 2), ('q2', 6), ('q3', 3), ('v1', 7), ('v2', 4), ('v2', 5), ('v3', 2), ('pra', 3)]),
    dict(jobs=[('q2', 7), ('q3', 4), ('q3', 5), ('v2', 6), ('v3', 3), ('postinv', 2), ('prb', 3)]),
    dict(jobs=[('inv', 3), ('q3', 6), ('v2', 7), ('v3', 4), ('v3', 5)]),
    dict(jobs=[('q3', 7), ('v3', 6), ('postinv', 3)]),
    dict(jobs=[('v3', 7)]),
]


def _kernel(keys,
            z_ref, u_hbm, are_hbm, aim_hbm, bre_hbm, bim_hbm, cre_hbm, cim_hbm, ldt_hbm, dsk_hbm,
            x_hbm, wqkv_hbm, wo_hbm, ctab_hbm,
            out_hbm,
            u_v, x_v, w_v, wo_v, ctab_v, par_v, ldt_v, dsk_v,
            dtc_v, g_v, h_v, rk_v, kt_v, rp_v, pk_v, v_v, zp_v, zrow_v, m_v,
            kp_v, ki_v, kx_v, kq_v, kr_v, zr_v, us_v, ua_v, ub_v, yh_v, ri_v,
            rq_v, pz_v, rd_v, o_v, ro_v,
            oa_v, ob_v, sems, osems):
    npair = len(keys)
    z = z_ref[0]

    def slot(name, mjobs, vjobs):
        seq = []
        mp = [p for j in mjobs for p in j]
        mt = sum(c for c, _ in mp) or 1
        acc = 0
        for c, f in mp:
            seq.append((acc / mt, 0, f))
            acc += c
        for j in vjobs:
            vt = sum(c for c, _ in j) or 1
            acc = 0
            for c, f in j:
                seq.append((acc / vt + 1e-6, 1, f))
                acc += c
        seq.sort(key=lambda e: (e[0], e[1]))
        with jax.named_scope(name):
            @pl.when(z == 0)
            def _():
                for _, _, f in seq:
                    f()

    def cp(src, dst, k):
        return pltpu.make_async_copy(src, dst, sems.at[k])

    cps_w = [cp(wqkv_hbm.at[:, pl.ds(128 * n, 128)], w_v.at[n], n) for n in range(12)]
    cps_x = [[cp(x_hbm.at[pl.ds(PR_ * rb, PR_), pl.ds(128 * kk, 128)], x_v.at[kk, pl.ds(PR_ * rb, PR_), :],
                 12 + 4 * rb + kk) for kk in range(4)] for rb in range(4)]
    cps_u = [cp(u_hbm.at[:, pl.ds(128 * j, 128)], u_v.at[j], 28 + j) for j in range(4)]
    cps_wo = [cp(wo_hbm.at[:, pl.ds(128 * n, 128)], wo_v.at[n], 32 + n) for n in range(4)]
    cp_c = cp(ctab_hbm, ctab_v, 36)
    par_hbm = (are_hbm, aim_hbm, bre_hbm, bim_hbm, cre_hbm, cim_hbm)
    cps_p0 = [cp(h.at[pl.ds(0, RB), :], par_v.at[i, pl.ds(0, RB), :], 37 + i) for i, h in enumerate(par_hbm)]
    cps_p1 = [cp(h.at[pl.ds(RB, D - RB), :], par_v.at[i, pl.ds(RB, D - RB), :], 43 + i) for i, h in enumerate(par_hbm)]
    cp_ldt = cp(ldt_hbm, ldt_v, 49)
    cp_dsk = cp(dsk_hbm, dsk_v, 50)
    order = ([cp_ldt] + cps_p0 + cps_x[0] + [cps_w[4], cps_w[8], cps_w[5], cps_w[9]] + cps_p1
             + [cps_w[6], cps_w[10], cps_w[7], cps_w[11]]
             + cps_x[1] + cps_x[2] + cps_x[3] + [cp_c] + cps_u + cps_w[:4] + cps_wo + [cp_dsk])
    for c in order:
        c.start()
    are_ref, aim_ref, bre_ref, bim_ref, cre_ref, cim_ref = (par_v.at[i] for i in range(6))

    xu, wu, uu, wou, cu = (r.bitcast(U32) for r in (x_v, w_v, u_v, wo_v, ctab_v))
    off_ffwd = npair * 256
    off_finv = off_ffwd + 256
    off_bm = off_finv + 256

    cp_ldt.wait()
    dt_row = jnp.exp(ldt_v[...].astype(F32).reshape(1, D)).astype(BF16).astype(F32)
    dtc_v[...] = jnp.transpose(jnp.broadcast_to(dt_row, (128, D)))

    def pre_k(t):
        def piece(q):
            if True:
                rows = slice(RB * t + 8 * q, RB * t + 8 * q + 8)
                dt = dtc_v[rows, :]
                lre = dt * are_ref[rows, :].astype(F32)
                lim = dt * aim_ref[rows, :].astype(F32)
                mag = jnp.exp(lre)
                p1 = (mag * jnp.cos(lim), mag * jnp.sin(lim))
                dbr = dt * bre_ref[rows, :].astype(F32)
                dbi = dt * bim_ref[rows, :].astype(F32)
                c0 = _cmul(cre_ref[rows, :].astype(F32), cim_ref[rows, :].astype(F32), dbr, dbi)
                pw = {1: p1}
                pw[2] = _cmul(*p1, *p1)
                pw[3] = _cmul(*pw[2], *p1)
                pw[4] = _cmul(*pw[2], *pw[2])
                pw[5] = _cmul(*pw[4], *p1)
                pw[6] = _cmul(*pw[4], *pw[2])
                pw[7] = _cmul(*pw[4], *pw[3])
                p8 = _cmul(*pw[4], *pw[4])
                h8 = (_rev8(p8[0]), _rev8(p8[1]))
                hs = [(jnp.ones((8, 128), F32), jnp.zeros((8, 128), F32)), h8]
                for b in range(2, 16):
                    hs.append(_cmul(*hs[-1], *h8))
                for b in range(0, 16, 2):
                    h_v[q, 0, 4 * b:4 * b + 8, :] = _pk(jnp.concatenate([hs[b][0], hs[b + 1][0]], axis=0))
                    h_v[q, 1, 4 * b:4 * b + 8, :] = _pk(jnp.concatenate([-hs[b][1], -hs[b + 1][1]], axis=0))
                p16 = _cmul(*p8, *p8)
                p32 = _cmul(*p16, *p16)
                p64 = _cmul(*p32, *p32)
                p128 = _cmul(*p64, *p64)
                zero = jnp.zeros((8, 128), F32)
                cur = c0
                curi = 0
                gs = []
                for e in ROW_E + [None]:
                    if e is None:
                        gs.append((zero, zero))
                    else:
                        i, rho = e // C, e % C
                        while curi < i:
                            cur = _cmul(*cur, *p128)
                            curi += 1
                        gs.append(cur if rho == 0 else _cmul(*cur, *pw[rho]))
                    if len(gs) % 2 == 0:
                        a = len(gs) - 2
                        g_v[q, 0, 4 * a:4 * a + 8, :] = _pk(jnp.concatenate([gs[a][0], gs[a + 1][0]], axis=0))
                        g_v[q, 1, 4 * a:4 * a + 8, :] = _pk(jnp.concatenate([gs[a][1], gs[a + 1][1]], axis=0))
        return [(850, functools.partial(piece, q)) for q in range(GPI)]

    def mxu_k(t):
        def piece(q2):
            for q in (2 * q2, 2 * q2 + 1):
                for hf in range(2):
                    rk_v[t % 2][q, hf] = _nt(pltpu.bitcast(g_v[q, hf], BF16), pltpu.bitcast(h_v[q, hf], BF16))
        return [(336, functools.partial(piece, q2)) for q2 in range(GPI // 2)]

    def post_k(t):
        def piece(q2):
            lane = lax.broadcasted_iota(jnp.int32, (8, 128), 1)
            r = rk_v[t % 2]
            if True:
                tiles = [[] for _ in range(6)]
                for q in (2 * q2, 2 * q2 + 1):
                    acc = [jnp.zeros((8, 128), F32)] * 6
                    for (tl, sl, a) in SLOTS:
                        o = r[q, 0, 8 * a:8 * a + 8, :] + r[q, 1, 8 * a:8 * a + 8, :]
                        rolled = pltpu.roll(o, sl + 1, 1, stride=1, stride_axis=0)
                        acc[tl] = jnp.where(lane % 8 == sl, rolled, acc[tl])
                    for tl in range(6):
                        tiles[tl].append(acc[tl])
                r0 = (RB * t + 16 * q2) // 2
                for tl in range(6):
                    kt_v[tl, r0:r0 + 8, :] = _pk(jnp.concatenate(tiles[tl], axis=0))
        return [(280, functools.partial(piece, q2)) for q2 in range(GPI // 2)]

    def proj(r0, nr, n, dst):
        for kk in range(4):
            dst[kk] = _nn(_ld(xu, kk, (r0, nr)), _ld(wu, n, (128 * kk, 128)))

    def mxu_p(i):
        rb, p = i // 4, i % 4
        return [(512, functools.partial(proj, PR_ * rb, PR_, 4 + p, rp_v[i % 4].at[0])),
                (512, functools.partial(proj, PR_ * rb, PR_, 8 + p, rp_v[i % 4].at[1]))]

    def post_p(i):
        def piece(c):
            rb, p = i // 4, i % 4
            r = rp_v[i % 4]
            zacc = None
            for r0 in range(64 * c, 64 * c + 64, 16):
                rs = slice(r0, r0 + 16)
                k = _phi((r[0, 0, rs, :] + r[0, 1, rs, :]) + (r[0, 2, rs, :] + r[0, 3, rs, :]))
                kb = k.astype(BF16)
                o8 = (PR_ * rb + r0) // 2
                pk_v[p, o8:o8 + 8, :] = pltpu.bitcast(kb, U32)
                kf = kb.astype(F32)
                zz = kf[:8] + kf[8:]
                zacc = zz if zacc is None else zacc + zz
                v_v[p, o8:o8 + 8, :] = _pk((r[1, 0, rs, :] + r[1, 1, rs, :]) + (r[1, 2, rs, :] + r[1, 3, rs, :]))
            zp_v[rb, p, c] = zacc
        return [(150, functools.partial(piece, c)) for c in range(PR_ // 64)]

    def kvm_piece(blk):
        bmask = _ld(cu, (off_bm, 128))
        if True:
            kv = _tn(_ld(pk_v, blk, (0, L)), _ld(v_v, blk, (0, L))) * bmask.astype(F32)
            kvb = kv.astype(BF16)
            for n in range(4):
                m_v[n, 64 * blk:64 * blk + 64, :] = _pk(_nn(kvb, _ld(wou, n, (128 * blk, 128))))
            zs = sum(zp_v[rb, blk, c] for rb in range(4) for c in range(8))
            zrow = jnp.sum(zs, axis=0, keepdims=True)
            zcol = jnp.transpose(jnp.broadcast_to(zrow, (128, 128)))
            zrow_v[blk] = _pk(zcol * bmask.astype(F32))

    def kvm():
        return [(650, functools.partial(kvm_piece, blk)) for blk in range(4)]

    main_pair = {}
    extra_pair = {}
    for pi, (al, tl) in enumerate(keys):
        if al in main_pair:
            extra_pair[al] = (pi, tl)
        else:
            main_pair[al] = (pi, tl)
    xidx = {al: i for i, al in enumerate(sorted(extra_pair))}

    def mxu_kh(j):
        def piece(c):
            for al in range(4 * c, 4 * c + 4):
                pi, tl = main_pair[al]
                r = _nt(_ld(cu, (256 * pi, 256)), _ld(kt_v, tl, (128 * j, 128)))
                kp_v[al, j] = r[:C]
                ki_v[al, j] = r[C:]
                if al in extra_pair:
                    pi, tl = extra_pair[al]
                    kx_v[xidx[al], j] = _nt(_ld(cu, (256 * pi, 256)), _ld(kt_v, tl, (128 * j, 128)))
        return [(304, functools.partial(piece, c)) for c in range(4)]

    def post_kh(j):
        def piece(c):
            for al in (c,):
                for r0 in range(0, C, 16):
                    rs = slice(r0, r0 + 16)
                    kr = kp_v[al, j, rs, :]
                    ki = ki_v[al, j, rs, :]
                    if al in extra_pair:
                        kr = kr + kx_v[xidx[al], j, rs, :]
                        ki = ki + kx_v[xidx[al], j, C + r0:C + r0 + 16, :]
                        kp_v[al, j, rs, :] = kr
                    kq_v[al, j, rs, :] = ki - kr
                    kr_v[al, j, rs, :] = kr + ki
        return [(40, functools.partial(piece, c)) for c in range(NCH)]

    def mxu_z(j):
        def piece(c):
            for a in range(4 * c, 4 * c + 4):
                zr_v[a, j] = _nn(_ld(cu, (off_ffwd, 256)), _ld(uu, j, (C * a, C)))
        return [(256, functools.partial(piece, c)) for c in range(4)]

    def post_z(j):
        def piece(c):
            for a in (c,):
                for r0 in range(0, C, 16):
                    rr = slice(r0, r0 + 16)
                    ri = slice(C + r0, C + r0 + 16)
                    zr, zi = zr_v[a, j, rr, :], zr_v[a, j, ri, :]
                    if a == 0:
                        ar, ai = (zi, -zr) if r0 < 64 else (-zi, zr)
                    elif r0 < 64:
                        ar, ai = zr_v[a - 1, j, rr, :] + zi, zr_v[a - 1, j, ri, :] - zr
                    else:
                        ar, ai = zr_v[a - 1, j, rr, :] - zi, zr_v[a - 1, j, ri, :] + zr
                    ua_v[a, j, rr, :] = ar
                    ub_v[a, j, rr, :] = ai
                    us_v[a, j, rr, :] = ar + ai
        return [(50, functools.partial(piece, c)) for c in range(NCH)]

    def prod_blk(j, kb, a0):
        rs = slice(8 * kb, 8 * kb + 8)
        acc = [[None] * 3 for _ in range(4)]
        uc = {}
        for al in range(a0 + 4):
            kk = (kp_v[al, j, rs, :], kq_v[al, j, rs, :], kr_v[al, j, rs, :])
            for o in range(4):
                ap = a0 + o - al
                if ap < 0:
                    continue
                if ap not in uc:
                    uc[ap] = (us_v[ap, j, rs, :], ua_v[ap, j, rs, :], ub_v[ap, j, rs, :])
                ux = uc[ap]
                for w in range(3):
                    tt = kk[w] * ux[w]
                    acc[o][w] = tt if acc[o][w] is None else acc[o][w] + tt
        return [(acc[o][0] - acc[o][2], acc[o][0] + acc[o][1]) for o in range(4)]

    def prod(j, kqs):
        def piece(kq, a0):
            r0 = prod_blk(j, 2 * kq, a0)
            r1 = prod_blk(j, 2 * kq + 1, a0)
            for o in range(4):
                a = a0 + o
                yh_v[a, j, 8 * kq:8 * kq + 8, :] = _pk(jnp.concatenate([r0[o][0], r1[o][0]], axis=0))
                yh_v[a, j, 64 + 8 * kq:64 + 8 * kq + 8, :] = _pk(jnp.concatenate([r0[o][1], r1[o][1]], axis=0))
        return [(12 * (4 * a0 + 10) + 30, functools.partial(piece, kq, a0)) for kq in kqs for a0 in range(0, NCH, 4)]

    def mxu_inv(j):
        def piece(c):
            for a in range(4 * c, 4 * c + 4):
                for hf in range(2):
                    ri_v[a, hf] = _nn(_ld(cu, (off_finv + 128 * hf, 128)), _ld(yh_v, a, j, (128 * hf, 128)))
        return [(256, functools.partial(piece, c)) for c in range(4)]

    def post_inv(j):
        def piece(c):
            dsk = dsk_v[...].astype(F32).reshape(1, D)[:, 128 * j:128 * j + 128]
            for a in (c,):
                for r0 in range(0, C, 16):
                    rs = slice(r0, r0 + 16)
                    y = ri_v[a, 0, rs, :] + ri_v[a, 1, rs, :]
                    ud = _ld(uu, j, (C * a + r0, 16)).astype(F32) * dsk
                    ya = y.astype(BF16).astype(F32) + ud.astype(BF16).astype(F32)
                    oa_v[j, C * a + r0:C * a + r0 + 16, :] = ya.astype(BF16)
        return [(90, functools.partial(piece, c)) for c in range(NCH)]

    def q1(i):
        return [(256, functools.partial(proj, QR * i, QR, n, rq_v[i % 4].at[n])) for n in range(4)]

    def v1(i):
        def piece(n, c):
            r = rq_v[i % 4]
            if True:
                for r0 in range(64 * c, 64 * c + 64, 16):
                    rs = slice(r0, r0 + 16)
                    pq = _phi((r[n, 0, rs, :] + r[n, 1, rs, :]) + (r[n, 2, rs, :] + r[n, 3, rs, :]))
                    pz_v[i, n, r0 // 2:r0 // 2 + 8, :] = _pk(pq)
        return [(100, functools.partial(piece, n, c)) for n in range(4) for c in range(QR // 64)]

    def q2(i):
        def piece():
            for n in range(4):
                rd_v[i, n] = _nn(pltpu.bitcast(pz_v[i, n], BF16), pltpu.bitcast(zrow_v[n], BF16))
        return [(256, piece)]

    def v2(i):
        def piece(n, c):
            if True:
                for r0 in range(64 * c, 64 * c + 64, 16):
                    rs = slice(r0, r0 + 16)
                    o_v[i, n, r0 // 2:r0 // 2 + 8, :] = _pk(_ld(pz_v, i, n, (r0, 16)).astype(F32) / (rd_v[i, n, rs, :] + 1e-6))
        return [(75, functools.partial(piece, n, c)) for n in range(4) for c in range(QR // 64)]

    def q3(i):
        def piece(n):
            if True:
                for kk in range(4):
                    ro_v[i % 4][n, kk] = _nn(pltpu.bitcast(o_v[i, kk], BF16), _ld(m_v, n, (128 * kk, 128)))
        return [(256, functools.partial(piece, n)) for n in range(4)]

    def v3(i):
        def piece(n, c):
            r = ro_v[i % 4]
            if True:
                for r0 in range(64 * c, 64 * c + 64, 16):
                    rs = slice(r0, r0 + 16)
                    ob_v[n, QR * i + r0:QR * i + r0 + 16, :] = (
                        (r[n, 0, rs, :] + r[n, 1, rs, :]) + (r[n, 2, rs, :] + r[n, 3, rs, :])).astype(BF16)
        return [(40, functools.partial(piece, n, c)) for n in range(4) for c in range(QR // 64)]

    ocopies = []

    def out_b(i):
        for n in range(4):
            c = pltpu.make_async_copy(ob_v.at[n, pl.ds(QR * i, QR), :],
                                      out_hbm.at[pl.ds(QR * i, QR), pl.ds(D + 128 * n, 128)], osems.at[4 * i + n])
            c.start()
            ocopies.append(c)

    def out_a(j):
        c = pltpu.make_async_copy(oa_v.at[j], out_hbm.at[:, pl.ds(128 * j, 128)], osems.at[4 * NQ + j])
        c.start()
        ocopies.append(c)

    def wait(cs):
        for c in cs:
            c.wait()

    A, B_ = [0, 1, 2, 3], [4, 5, 6, 7]
    jobs = dict(preka=lambda t: pre_k(t)[:4], prekb=lambda t: pre_k(t)[4:], mk=mxu_k, mp=mxu_p, prek=pre_k, postk=post_k, postp=post_p, kvm=lambda: kvm(), kh=mxu_kh,
                postkh=post_kh, z=mxu_z, postz=post_z, pra=lambda j: prod(j, A), prb=lambda j: prod(j, B_),
                inv=mxu_inv, postinv=post_inv, q1=q1, v1=v1, q2=q2, v2=v2, q3=q3, v3=v3)
    MXU_JOBS = ('mk', 'mp', 'kvm', 'kh', 'z', 'inv', 'q1', 'q2', 'q3')

    def deps(name, *a):
        i = a[0] if a else None
        return {
            'mk': lambda: [('prek', i)] if i else [('preka', 0), ('prekb', 0)],
            'postk': lambda: [('mk', i)],
            'postp': lambda: [('mp', i)],
            'kvm': lambda: [('postp', k) for k in range(16)],
            'kh': lambda: [('postk', 2 * i), ('postk', 2 * i + 1)],
            'postkh': lambda: [('kh', i)],
            'postz': lambda: [('z', i)],
            'pra': lambda: [('postkh', i), ('postz', i)],
            'prb': lambda: [('postkh', i), ('postz', i)],
            'inv': lambda: [('pra', i), ('prb', i)],
            'postinv': lambda: [('inv', i)],
            'v1': lambda: [('q1', i)],
            'q2': lambda: [('v1', i), ('kvm',)],
            'v2': lambda: [('q2', i)],
            'q3': lambda: [('v2', i), ('kvm',)],
            'v3': lambda: [('q3', i)],
        }.get(name, lambda: [])()

    table = SCHEDULE
    done = {}
    for si, entry in enumerate(table):
        for job in entry['jobs']:
            for d in deps(*job):
                assert d in done and done[d] < si, (si, job, d)
        for job in entry['jobs']:
            done[job] = si
    waits = dict(x0=cps_x[0], x1=cps_x[1], x2=cps_x[2], x3=cps_x[3],
                 wa=[cps_w[4], cps_w[8], cps_w[5], cps_w[9]], wb=[cps_w[6], cps_w[10], cps_w[7], cps_w[11]],
                 c=[cp_c], u=cps_u, wq=cps_w[:4], wo=cps_wo + [cp_dsk], p0=cps_p0, p1=cps_p1)
    for si, entry in enumerate(table):
        for w in entry.get('wait', ()):
            wait(waits[w])
        mj = [jobs[j[0]](*j[1:]) for j in entry['jobs'] if j[0] in MXU_JOBS]
        vj = [jobs[j[0]](*j[1:]) for j in entry['jobs'] if j[0] not in MXU_JOBS]
        slot('s%d' % si, mj, vj)
        for j in entry['jobs']:
            if j[0] == 'v3':
                out_b(j[1])
            if j[0] == 'postinv':
                out_a(j[1])
    wait(ocopies)


@jax.jit
def pallas_concat_heads__ssm_conv_s4__linear_attn_block__prompt_kernel(
    A_u: jax.Array,
    A_A_re: jax.Array,
    A_A_im: jax.Array,
    A_B_re: jax.Array,
    A_B_im: jax.Array,
    A_C_re: jax.Array,
    A_C_im: jax.Array,
    A_log_dt: jax.Array,
    A_Dskip: jax.Array,
    B_x: jax.Array,
    B_wqkv: jax.Array,
    B_wo: jax.Array,
):
    keys, ctab = _constants()
    any_spec = pl.BlockSpec(memory_space=pl.ANY)
    vm = pl.BlockSpec(memory_space=pltpu.VMEM)
    V = pltpu.VMEM

    out = pl.pallas_call(
        functools.partial(_kernel, keys),
        out_shape=jax.ShapeDtypeStruct((L, 2 * D), BF16),
        in_specs=[pl.BlockSpec(memory_space=pltpu.SMEM)] + [any_spec] * 13,
        out_specs=any_spec,
        scratch_shapes=[
            V((4, L, 128), BF16),
            V((4, L, 128), BF16),
            V((12, D, 128), BF16),
            V((4, D, 128), BF16),
            V(ctab.shape, BF16),
            V((6, D, 128), BF16),
            V((D,), BF16),
            V((D,), BF16),
            V((D, 128), F32),
            V((GPI, 2, GROWS // 2, 128), U32),
            V((GPI, 2, 64, 128), U32),
            [V((GPI, 2, GROWS, 128), F32)] * 2,
            V((6, D // 2, 128), U32),
            [V((2, 4, PR_, 128), F32)] * 4,
            V((4, L // 2, 128), U32),
            V((4, L // 2, 128), U32),
            V((4, 4, 8, 8, 128), F32),
            V((4, 64, 128), U32),
            V((4, D // 2, 128), U32),
            V((NCH, ND, C, 128), F32),
            V((NCH, ND, C, 128), F32),
            V((3, ND, 2 * C, 128), F32),
            V((NCH, ND, C, 128), F32),
            V((NCH, ND, C, 128), F32),
            V((NCH, ND, 2 * C, 128), F32),
            V((NCH, ND, C, 128), F32),
            V((NCH, ND, C, 128), F32),
            V((NCH, ND, C, 128), F32),
            V((NCH, ND, C, 128), U32),
            V((NCH, 2, C, 128), F32),
            [V((4, 4, QR, 128), F32)] * 4,
            V((NQ, 4, QR // 2, 128), U32),
            V((NQ, 4, QR, 128), F32),
            V((NQ, 4, QR // 2, 128), U32),
            [V((4, 4, QR, 128), F32)] * 4,
            V((4, L, 128), BF16),
            V((4, L, 128), BF16),
            pltpu.SemaphoreType.DMA((51,)),
            pltpu.SemaphoreType.DMA((4 * NQ + 4,)),
        ],
        compiler_params=pltpu.CompilerParams(vmem_limit_bytes=120 * 1024 * 1024),
    )(
        jnp.zeros((1,), jnp.int32),
        A_u.reshape(L, D), A_A_re, A_A_im, A_B_re, A_B_im, A_C_re, A_C_im,
        A_log_dt, A_Dskip,
        B_x.reshape(L, D), B_wqkv, B_wo, jnp.asarray(ctab),
    )
    return out.reshape(1, L, 2 * D)
```

```python
import functools

import numpy as np
import jax
import jax.numpy as jnp
from jax import lax
import jax.experimental.pallas as pl
import jax.experimental.pallas.tpu as pltpu

L = 2048
D = 512
NS = 128
C = 128
NCH = L // C
H = 32
DH = D // H
ND = D // 128

F32 = jnp.float32
BF16 = jnp.bfloat16
U32 = jnp.uint32


PAIRS = [(0, 4), (1, 5), (2, 6), (3, 7), (256, 512), (258, 516), (260, 768), (262, 772),
         (1024, 2048), (1280, 512), (1536, 1024), (1792, None)]
NP_ = len(PAIRS)
GROWS = 8 * NP_
NB = 32


def _lane(a_lo, b, slot):
    return 4 * ((b + 1 + a_lo) % NB) + slot


@functools.lru_cache(maxsize=None)
def _constants():
    bf = jnp.bfloat16
    rl = np.arange(L).astype(np.float32).astype(bf).astype(np.int64)
    kperm = np.concatenate([np.arange(0, C, 2), np.arange(1, C, 2)])

    def w(j):
        return np.exp(-1j * np.pi * (2 * kperm + 1) * j / 256.0)

    def main_tiles(al):
        return [0, 3] if al < 2 else [1] if al < 4 else [4] if al < 8 else [2]

    pairs = {}
    for al in range(NCH):
        for j in range(C):
            v = int(rl[C * al + j])
            found = None
            for tl in main_tiles(al) + [5]:
                a_lo, mu = tl // 3, tl % 3
                for slot in range(4):
                    e = PAIRS[4 * mu + slot][a_lo]
                    if e is not None and v >= e and (v - e) % 8 == 0 and (v - e) // 8 < NB:
                        found = (tl, _lane(a_lo, (v - e) // 8, slot))
                        break
                if found:
                    break
            m = pairs.setdefault((al, found[0]), np.zeros((C, C), np.complex128))
            m[:, found[1]] += w(j)
    keys = sorted(pairs.keys())
    fsel = np.stack([np.concatenate([pairs[k].real, pairs[k].imag], 0) for k in keys])
    ff = np.stack([w(j) for j in range(C)], 1)
    ffwd = np.concatenate([ff.real, ff.imag], 0)
    tau = np.arange(C)
    ang = 2 * np.pi * (kperm[None, :] + 0.5) * (C + tau[:, None]) / 256.0
    fre, fim = np.cos(ang) * (2.0 / 256.0), -np.sin(ang) * (2.0 / 256.0)
    finv = np.zeros((2, 128, 128))
    for kb in range(16):
        h, o = kb // 8, 16 * (kb % 8)
        finv[h, :, o:o + 8] = fre[:, 8 * kb:8 * kb + 8]
        finv[h, :, o + 8:o + 16] = fim[:, 8 * kb:8 * kb + 8]
    hid = np.arange(128) // DH
    bmask = (hid[:, None] == hid[None, :]).astype(np.float32)
    tab = np.concatenate([fsel.reshape(-1, 128), ffwd, finv.reshape(-1, 128), bmask], 0)
    return tuple(keys), tab.astype(bf)


def _cmul(ar, ai, br, bi):
    return ar * br - ai * bi, ar * bi + ai * br


def _nt(a, b):
    return lax.dot_general(a, b, (((1,), (1,)), ((), ())), preferred_element_type=F32)


def _tn(a, b):
    return lax.dot_general(a, b, (((0,), (0,)), ((), ())), preferred_element_type=F32)


def _nn(a, b):
    return jnp.dot(a, b, preferred_element_type=F32)


def _phi(t):
    return jnp.where(t > 0, t + 1.0, jnp.exp(t)) + 1e-6


def _ld(ref_u32, *idx):
    *lead, (r0, n) = idx
    return pltpu.bitcast(ref_u32[(*lead, slice(r0 // 2, (r0 + n) // 2), slice(None))], BF16)


def _pk(x):
    return pltpu.bitcast(x.astype(BF16), U32)


def _sincos(x):
    n = jnp.round(x * 0.6366197723675814)
    r = x - n * 1.5703125
    r = r - n * 4.837512969970703e-04
    r = r - n * 7.549789954891882e-08
    r2 = r * r
    sp = r + r * r2 * (-1.6666654611e-01 + r2 * (8.3321608736e-03 + r2 * (-1.9515295891e-04)))
    cp = 1.0 - 0.5 * r2 + r2 * r2 * (4.166664568298827e-02 + r2 * (-1.388731625493765e-03 + r2 * 2.443315711809948e-05))
    q = n.astype(jnp.int32)
    swap = (q & 1) == 1
    sn = jnp.where(swap, cp, sp)
    cs = jnp.where(swap, sp, cp)
    sn = jnp.where((q & 2) == 2, -sn, sn)
    cs = jnp.where(((q + 1) & 2) == 2, -cs, cs)
    return sn, cs


def _rev4(x):
    sub = lax.broadcasted_iota(jnp.int32, x.shape, 0)
    for bit in (2, 1):
        up = pltpu.roll(x, 8 - bit, 0)
        dn = pltpu.roll(x, bit, 0)
        x = jnp.where((sub & bit) == 0, up, dn)
    return x


GPI = 8
RB = 8 * GPI
NKI = D // RB
PR_ = 512
QR = 256
NQ = L // QR


SCHEDULE = [
    dict(wait=['p0'], jobs=[('preka', 0)]),
    dict(wait=['x0', 'wa'], jobs=[('mp', 0), ('mp', 1), ('prekb', 0)]),
    dict(wait=['wb', 'p1'], jobs=[('mk', 0), ('mp', 2), ('mp', 3), ('postp', 0), ('postp', 1), ('prek', 1)]),
    dict(wait=['x1'], jobs=[('mk', 1), ('mp', 4), ('mp', 5), ('postk', 0), ('postp', 2), ('postp', 3), ('prek', 2)]),
    dict(jobs=[('mk', 2), ('mp', 6), ('mp', 7), ('postk', 1), ('postp', 4), ('postp', 5), ('prek', 3)]),
    dict(wait=['x2'], jobs=[('mk', 3), ('mp', 8), ('mp', 9), ('postk', 2), ('postp', 6), ('postp', 7), ('prek', 4)]),
    dict(jobs=[('mk', 4), ('mp', 10), ('mp', 11), ('postk', 3), ('postp', 8), ('postp', 9), ('prek', 5)]),
    dict(wait=['x3'], jobs=[('mk', 5), ('mp', 12), ('mp', 13), ('postk', 4), ('postp', 10), ('postp', 11), ('prek', 6)]),
    dict(jobs=[('mk', 6), ('mp', 14), ('mp', 15), ('postk', 5), ('postp', 12), ('postp', 13), ('prek', 7)]),
    dict(wait=['c', 'u'], jobs=[('mk', 7), ('kh', 0), ('z', 0), ('postk', 6), ('postp', 14), ('postp', 15)]),
    dict(wait=['wq', 'wo'], jobs=[('kvm',), ('kh', 1), ('q1', 0), ('postk', 7)]),
    dict(jobs=[('z', 1), ('kh', 2), ('q1', 1), ('v1', 0), ('pra', 0)]),
    dict(jobs=[('z', 2), ('q2', 0), ('q1', 2), ('kh', 3), ('v1', 1), ('prb', 0)]),
    dict(jobs=[('inv', 0), ('z', 3), ('q1', 3), ('q2', 1), ('v1', 2), ('v2', 0), ('pra', 1)]),
    dict(jobs=[('q1', 4), ('q2', 2), ('q3', 0), ('q1', 5), ('v1', 3), ('v2', 1), ('postinv', 0), ('prb', 1)]),
    dict(jobs=[('inv', 1), ('q2', 3), ('q3', 1), ('q1', 6), ('v1', 4), ('v1', 5), ('v2', 2), ('v3', 0), ('pra', 2)]),
    dict(jobs=[('q1', 7), ('q2', 4), ('q2', 5), ('q3', 2), ('v1', 6), ('v2', 3), ('v3', 1), ('postinv', 1), ('prb', 2)]),
    dict(jobs=[('inv', 2), ('q2', 6), ('q3', 3), ('v1', 7), ('v2', 4), ('v2', 5), ('v3', 2), ('pra', 3)]),
    dict(jobs=[('q2', 7), ('q3', 4), ('q3', 5), ('v2', 6), ('v3', 3), ('postinv', 2), ('prb', 3)]),
    dict(jobs=[('inv', 3), ('q3', 6), ('v2', 7), ('v3', 4), ('v3', 5)]),
    dict(jobs=[('q3', 7), ('v3', 6), ('postinv', 3)]),
    dict(jobs=[('v3', 7)]),
]


def _kernel(keys,
            z_ref, u_hbm, are_hbm, aim_hbm, bre_hbm, bim_hbm, cre_hbm, cim_hbm, ldt_hbm, dsk_hbm,
            x_hbm, wqkv_hbm, wo_hbm, ctab_hbm,
            out_hbm,
            u_v, x_v, w_v, wo_v, ctab_v, par_v, ldt_v, dsk_v,
            dtc_v, g_v, h_v, rk_v, kt_v, rp_v, pk_v, v_v, zp_v, zrow_v, m_v,
            kp_v, ki_v, kx_v, zr_v, yh_v, ri_v,
            rq_v, pz_v, rd_v, o_v, ro_v,
            oa_v, ob_v, sems, osems):
    npair = len(keys)
    z = z_ref[0]

    def slot(name, mjobs, vjobs):
        seq = []
        mp = [p for j in mjobs for p in j]
        mt = sum(c for c, _ in mp) or 1
        acc = 0
        for c, f in mp:
            seq.append((acc / mt, 0, f))
            acc += c
        for j in vjobs:
            vt = sum(c for c, _ in j) or 1
            acc = 0
            for c, f in j:
                seq.append((acc / vt + 1e-6, 1, f))
                acc += c
        seq.sort(key=lambda e: (e[0], e[1]))
        with jax.named_scope(name):
            @pl.when(z == 0)
            def _():
                for _, _, f in seq:
                    f()

    def cp(src, dst, k):
        return pltpu.make_async_copy(src, dst, sems.at[k])

    cps_w = [cp(wqkv_hbm.at[:, pl.ds(128 * n, 128)], w_v.at[n], n) for n in range(12)]
    cps_x = [[cp(x_hbm.at[pl.ds(PR_ * rb, PR_), pl.ds(128 * kk, 128)], x_v.at[kk, pl.ds(PR_ * rb, PR_), :],
                 12 + 4 * rb + kk) for kk in range(4)] for rb in range(4)]
    cps_u = [cp(u_hbm.at[:, pl.ds(128 * j, 128)], u_v.at[j], 28 + j) for j in range(4)]
    cps_wo = [cp(wo_hbm.at[:, pl.ds(128 * n, 128)], wo_v.at[n], 32 + n) for n in range(4)]
    cp_c = cp(ctab_hbm, ctab_v, 36)
    par_hbm = (are_hbm, aim_hbm, bre_hbm, bim_hbm, cre_hbm, cim_hbm)
    cps_p0 = [cp(h.at[pl.ds(0, RB), :], par_v.at[i, pl.ds(0, RB), :], 37 + i) for i, h in enumerate(par_hbm)]
    cps_p1 = [cp(h.at[pl.ds(RB, D - RB), :], par_v.at[i, pl.ds(RB, D - RB), :], 43 + i) for i, h in enumerate(par_hbm)]
    cp_ldt = cp(ldt_hbm, ldt_v, 49)
    cp_dsk = cp(dsk_hbm, dsk_v, 50)
    order = ([cp_ldt] + cps_p0 + cps_x[0] + [cps_w[4], cps_w[8], cps_w[5], cps_w[9]] + cps_p1
             + [cps_w[6], cps_w[10], cps_w[7], cps_w[11]]
             + cps_x[1] + cps_x[2] + cps_x[3] + [cp_c] + cps_u + cps_w[:4] + cps_wo + [cp_dsk])
    for c in order:
        c.start()
    are_ref, aim_ref, bre_ref, bim_ref, cre_ref, cim_ref = (par_v.at[i] for i in range(6))

    xu, wu, uu, wou, cu = (r.bitcast(U32) for r in (x_v, w_v, u_v, wo_v, ctab_v))
    off_ffwd = npair * 256
    off_finv = off_ffwd + 256
    off_bm = off_finv + 256

    cp_ldt.wait()
    dt_row = jnp.exp(ldt_v[...].astype(F32).reshape(1, D)).astype(BF16).astype(F32)
    dtc_v[...] = jnp.transpose(jnp.broadcast_to(dt_row, (128, D)))

    def pre_k(t):
        def gen(q):
            rows = slice(RB * t + 8 * q, RB * t + 8 * q + 8)
            dt = dtc_v[rows, :]
            lre = dt * are_ref[rows, :].astype(F32)
            lim = dt * aim_ref[rows, :].astype(F32)
            mag = jnp.exp(lre)
            sn, cs = _sincos(lim)
            p1 = (mag * cs, mag * sn)
            dbr = dt * bre_ref[rows, :].astype(F32)
            dbi = dt * bim_ref[rows, :].astype(F32)
            c0 = _cmul(cre_ref[rows, :].astype(F32), cim_ref[rows, :].astype(F32), dbr, dbi)
            yield
            pw = {1: p1}
            pw[2] = _cmul(*p1, *p1)
            yield
            pw[3] = _cmul(*pw[2], *p1)
            pw[4] = _cmul(*pw[2], *pw[2])
            yield
            pw[5] = _cmul(*pw[4], *p1)
            pw[6] = _cmul(*pw[4], *pw[2])
            pw[7] = _cmul(*pw[4], *pw[3])
            p8 = _cmul(*pw[4], *pw[4])
            yield
            low = lax.broadcasted_iota(jnp.int32, (8, 128), 0) < 4

            def emit(dst, part, idx, pend, a, b):
                pend.append((jnp.where(low, a, pltpu.roll(b, 4, 0)), jnp.where(low, pltpu.roll(a, 4, 0), b)))
                if len(pend) == 2:
                    r0 = 8 * (idx // 2)
                    dst[q, 0, part, r0:r0 + 8, :] = _pk(jnp.concatenate([pend[0][0], pend[1][0]], axis=0))
                    dst[q, 1, part, r0:r0 + 8, :] = _pk(jnp.concatenate([pend[0][1], pend[1][1]], axis=0))
                    pend.clear()

            p16 = _cmul(*p8, *p8)
            h8 = (_rev4(p8[0]), -_rev4(p8[1]))
            h16 = _cmul(*h8, *h8)
            yield
            p32 = _cmul(*p16, *p16)
            yield
            p64 = _cmul(*p32, *p32)
            yield
            p128 = _cmul(*p64, *p64)
            yield
            p256 = _cmul(*p128, *p128)
            yield
            zero = jnp.zeros((8, 128), F32)
            gt = {0: c0, None: (zero, zero)}

            def grow(e):
                if e not in gt:
                    if e % 256 == 0:
                        gt[e] = _cmul(*grow(e - 256), *p256)
                    else:
                        gt[e] = _cmul(*grow(256 * (e // 256)), *pw[e % 256])
                return gt[e]

            h0 = (jnp.ones((8, 128), F32), jnp.zeros((8, 128), F32))
            hr, hi_, gr, gi = [], [], [], []
            for be in range(NB // 2):
                h1 = h8 if be == 0 else _cmul(*h0, *h8)
                hn = None
                if be + 1 < NB // 2:
                    hn = h16 if be == 0 else _cmul(*h0, *h16)
                emit(h_v, 0, be, hr, h0[0], h1[0])
                emit(h_v, 1, be, hi_, h0[1], h1[1])
                h0 = hn
                if be < NP_:
                    a, b = grow(PAIRS[be][0]), grow(PAIRS[be][1])
                    emit(g_v, 0, be, gr, a[0], b[0])
                    emit(g_v, 1, be, gi, a[1], b[1])
                yield

        def piece(q2):
            gens = [gen(2 * q2), gen(2 * q2 + 1)]
            while gens:
                for g in list(gens):
                    try:
                        next(g)
                    except StopIteration:
                        gens.remove(g)
        return [(1600, functools.partial(piece, q2)) for q2 in range(GPI // 2)]

    def mxu_k(t):
        def piece(q2):
            for q in (2 * q2, 2 * q2 + 1):
                for par in range(2):
                    for hf in range(2):
                        rk_v[t % 2][q, par, hf] = _nt(pltpu.bitcast(g_v[q, par, hf], BF16),
                                                      pltpu.bitcast(h_v[q, par, hf], BF16))
        return [(192, functools.partial(piece, q2)) for q2 in range(GPI // 2)]

    def post_k(t):
        def piece(q2):
            lane = lax.broadcasted_iota(jnp.int32, (8, 128), 1)
            low = lax.broadcasted_iota(jnp.int32, (8, 128), 0) < 4
            r = rk_v[t % 2]
            tiles = [[] for _ in range(6)]
            for q in (2 * q2, 2 * q2 + 1):
                acc = [[jnp.zeros((8, 128), F32)] * 3 for _ in range(2)]
                for par in range(2):
                    for pp in range(NP_):
                        mu, sl = pp // 4, pp % 4
                        o = r[q, par, 0, 8 * pp:8 * pp + 8, :] + r[q, par, 1, 8 * pp:8 * pp + 8, :]
                        rolled = pltpu.roll(o, sl + 1, 1, stride=1, stride_axis=0)
                        acc[par][mu] = jnp.where(lane % 4 == sl, rolled, acc[par][mu])
                for mu in range(3):
                    x, y = acc[0][mu], acc[1][mu]
                    tiles[mu].append(jnp.where(low, x, pltpu.roll(y, 4, 0)))
                    tiles[3 + mu].append(jnp.where(low, pltpu.roll(x, 4, 0), y))
            r0 = (RB * t + 16 * q2) // 2
            for tl in range(6):
                kt_v[tl, r0:r0 + 8, :] = _pk(jnp.concatenate(tiles[tl], axis=0))
        return [(190, functools.partial(piece, q2)) for q2 in range(GPI // 2)]

    def proj(r0, nr, n, dst):
        for kk in range(4):
            dst[kk] = _nn(_ld(xu, kk, (r0, nr)), _ld(wu, n, (128 * kk, 128)))

    def mxu_p(i):
        rb, p = i // 4, i % 4
        return [(512, functools.partial(proj, PR_ * rb, PR_, 4 + p, rp_v[i % 4].at[0])),
                (512, functools.partial(proj, PR_ * rb, PR_, 8 + p, rp_v[i % 4].at[1]))]

    def post_p(i):
        def piece(c):
            rb, p = i // 4, i % 4
            r = rp_v[i % 4]
            zacc = None
            for r0 in range(64 * c, 64 * c + 64, 16):
                rs = slice(r0, r0 + 16)
                k = _phi((r[0, 0, rs, :] + r[0, 1, rs, :]) + (r[0, 2, rs, :] + r[0, 3, rs, :]))
                kb = k.astype(BF16)
                o8 = (PR_ * rb + r0) // 2
                pk_v[p, o8:o8 + 8, :] = pltpu.bitcast(kb, U32)
                zz = k[:8] + k[8:]
                zacc = zz if zacc is None else zacc + zz
                v_v[p, o8:o8 + 8, :] = _pk((r[1, 0, rs, :] + r[1, 1, rs, :]) + (r[1, 2, rs, :] + r[1, 3, rs, :]))
            zp_v[rb, p, c] = zacc
        return [(150, functools.partial(piece, c)) for c in range(PR_ // 64)]

    def kvm_piece(blk):
        bmask = _ld(cu, (off_bm, 128))
        if True:
            kv = _tn(_ld(pk_v, blk, (0, L)), _ld(v_v, blk, (0, L))) * bmask.astype(F32)
            kvb = kv.astype(BF16)
            for n in range(4):
                m_v[n, 64 * blk:64 * blk + 64, :] = _pk(_nn(kvb, _ld(wou, n, (128 * blk, 128))))
            zs = sum(zp_v[rb, blk, c] for rb in range(4) for c in range(8))
            zrow = jnp.sum(zs, axis=0, keepdims=True)
            zcol = jnp.transpose(jnp.broadcast_to(zrow, (128, 128)))
            zrow_v[blk] = _pk(zcol * bmask.astype(F32))

    def kvm():
        return [(650, functools.partial(kvm_piece, blk)) for blk in range(4)]

    main_pair = {}
    extra_pair = {}
    for pi, (al, tl) in enumerate(keys):
        if al in main_pair:
            extra_pair[al] = (pi, tl)
        else:
            main_pair[al] = (pi, tl)
    xidx = {al: i for i, al in enumerate(sorted(extra_pair))}

    def mxu_kh(j):
        def piece(c):
            for al in range(4 * c, 4 * c + 4):
                pi, tl = main_pair[al]
                r = _nt(_ld(cu, (256 * pi, 256)), _ld(kt_v, tl, (128 * j, 128)))
                kp_v[al, j] = r[:C]
                ki_v[al, j] = r[C:]
                if al in extra_pair:
                    pi, tl = extra_pair[al]
                    kx_v[xidx[al], j] = _nt(_ld(cu, (256 * pi, 256)), _ld(kt_v, tl, (128 * j, 128)))
        return [(336, functools.partial(piece, c)) for c in range(4)]

    def post_kh(j):
        def piece(c):
            for al in (c,):
                for r0 in range(0, C, 16):
                    rs = slice(r0, r0 + 16)
                    kr = kp_v[al, j, rs, :]
                    ki = ki_v[al, j, rs, :]
                    if al in extra_pair:
                        kr = kr + kx_v[xidx[al], j, rs, :]
                        ki = ki + kx_v[xidx[al], j, C + r0:C + r0 + 16, :]
                        kp_v[al, j, rs, :] = kr
                    kq_v[al, j, rs, :] = ki - kr
                    kr_v[al, j, rs, :] = kr + ki
        return [(40, functools.partial(piece, c)) for c in range(NCH)]

    def mxu_z(j):
        def piece(c):
            for a in range(4 * c, 4 * c + 4):
                zr_v[a, j] = _nn(_ld(cu, (off_ffwd, 256)), _ld(uu, j, (C * a, C)))
        return [(256, functools.partial(piece, c)) for c in range(4)]

    def post_z(j):
        def piece(c):
            for a in (c,):
                for r0 in range(0, C, 16):
                    rr = slice(r0, r0 + 16)
                    ri = slice(C + r0, C + r0 + 16)
                    zr, zi = zr_v[a, j, rr, :], zr_v[a, j, ri, :]
                    if a == 0:
                        ar, ai = (zi, -zr) if r0 < 64 else (-zi, zr)
                    elif r0 < 64:
                        ar, ai = zr_v[a - 1, j, rr, :] + zi, zr_v[a - 1, j, ri, :] - zr
                    else:
                        ar, ai = zr_v[a - 1, j, rr, :] - zi, zr_v[a - 1, j, ri, :] + zr
                    ua_v[a, j, rr, :] = ar
                    ub_v[a, j, rr, :] = ai
                    us_v[a, j, rr, :] = ar + ai
        return [(50, functools.partial(piece, c)) for c in range(NCH)]

    def prod_blk(j, kb, a0):
        rs = slice(8 * kb, 8 * kb + 8)
        ri = slice(C + 8 * kb, C + 8 * kb + 8)
        acc = [[None] * 3 for _ in range(4)]
        uc = {}
        zc = {}

        def zraw(a):
            if a not in zc:
                zc[a] = (zr_v[a, j, rs, :], zr_v[a, j, ri, :])
            return zc[a]

        for al in range(a0 + 4):
            kr, ki = kp_v[al, j, rs, :], ki_v[al, j, rs, :]
            if al in extra_pair:
                kr = kr + kx_v[xidx[al], j, rs, :]
                ki = ki + kx_v[xidx[al], j, ri, :]
            kk = (kr, ki - kr, kr + ki)
            for o in range(3, -1, -1):
                ap = a0 + o - al
                if ap < 0:
                    continue
                if ap not in uc:
                    zr, zi = zraw(ap)
                    if ap == 0:
                        ar, ai = (zi, -zr) if kb < 8 else (-zi, zr)
                    else:
                        pr, pi = zraw(ap - 1)
                        ar, ai = (pr + zi, pi - zr) if kb < 8 else (pr - zi, pi + zr)
                    uc[ap] = (ar + ai, ar, ai)
                ux = uc[ap]
                for w in range(3):
                    tt = kk[w] * ux[w]
                    acc[o][w] = tt if acc[o][w] is None else acc[o][w] + tt
        return [(acc[o][0] - acc[o][2], acc[o][0] + acc[o][1]) for o in range(4)]

    def prod(j, kbs):
        def piece(kb, a0):
            r = prod_blk(j, kb, a0)
            for o in range(4):
                yh_v[a0 + o, j, 8 * kb:8 * kb + 8, :] = _pk(jnp.concatenate([r[o][0], r[o][1]], axis=0))
        return [(6 * (4 * a0 + 10) + 5 * (a0 + 4) + 15, functools.partial(piece, kb, a0)) for kb in kbs for a0 in range(0, NCH, 4)]

    def mxu_inv(j):
        def piece(c):
            for a in range(4 * c, 4 * c + 4):
                for hf in range(2):
                    ri_v[a, hf] = _nn(_ld(cu, (off_finv + 128 * hf, 128)), _ld(yh_v, a, j, (128 * hf, 128)))
        return [(256, functools.partial(piece, c)) for c in range(4)]

    def post_inv(j):
        def piece(c):
            dsk = dsk_v[...].astype(F32).reshape(1, D)[:, 128 * j:128 * j + 128]
            for a in (c,):
                for r0 in range(0, C, 16):
                    rs = slice(r0, r0 + 16)
                    y = ri_v[a, 0, rs, :] + ri_v[a, 1, rs, :]
                    ud = _ld(uu, j, (C * a + r0, 16)).astype(F32) * dsk
                    oa_v[j, C * a + r0:C * a + r0 + 16, :] = (y + ud).astype(BF16)
        return [(90, functools.partial(piece, c)) for c in range(NCH)]

    def q1(i):
        return [(256, functools.partial(proj, QR * i, QR, n, rq_v[i % 4].at[n])) for n in range(4)]

    def v1(i):
        def piece(n, c):
            r = rq_v[i % 4]
            if True:
                for r0 in range(64 * c, 64 * c + 64, 16):
                    rs = slice(r0, r0 + 16)
                    pq = _phi((r[n, 0, rs, :] + r[n, 1, rs, :]) + (r[n, 2, rs, :] + r[n, 3, rs, :]))
                    pz_v[i, n, r0 // 2:r0 // 2 + 8, :] = _pk(pq)
        return [(100, functools.partial(piece, n, c)) for n in range(4) for c in range(QR // 64)]

    def q2(i):
        def piece():
            for n in range(4):
                rd_v[i, n] = _nn(pltpu.bitcast(pz_v[i, n], BF16), pltpu.bitcast(zrow_v[n], BF16))
        return [(256, piece)]

    def v2(i):
        def piece(n, c):
            if True:
                for r0 in range(64 * c, 64 * c + 64, 16):
                    rs = slice(r0, r0 + 16)
                    o_v[i, n, r0 // 2:r0 // 2 + 8, :] = _pk(_ld(pz_v, i, n, (r0, 16)).astype(F32) * pl.reciprocal(rd_v[i, n, rs, :] + 1e-6, approx=True))
        return [(75, functools.partial(piece, n, c)) for n in range(4) for c in range(QR // 64)]

    def q3(i):
        def piece(n):
            if True:
                for kk in range(4):
                    ro_v[i % 4][n, kk] = _nn(pltpu.bitcast(o_v[i, kk], BF16), _ld(m_v, n, (128 * kk, 128)))
        return [(256, functools.partial(piece, n)) for n in range(4)]

    def v3(i):
        def piece(n, c):
            r = ro_v[i % 4]
            if True:
                for r0 in range(64 * c, 64 * c + 64, 16):
                    rs = slice(r0, r0 + 16)
                    ob_v[n, QR * i + r0:QR * i + r0 + 16, :] = (
                        (r[n, 0, rs, :] + r[n, 1, rs, :]) + (r[n, 2, rs, :] + r[n, 3, rs, :])).astype(BF16)
        return [(40, functools.partial(piece, n, c)) for n in range(4) for c in range(QR // 64)]

    ocopies = []

    def out_b(i):
        for n in range(4):
            c = pltpu.make_async_copy(ob_v.at[n, pl.ds(QR * i, QR), :],
                                      out_hbm.at[pl.ds(QR * i, QR), pl.ds(D + 128 * n, 128)], osems.at[4 * i + n])
            c.start()
            ocopies.append(c)

    def out_a(j):
        c = pltpu.make_async_copy(oa_v.at[j], out_hbm.at[:, pl.ds(128 * j, 128)], osems.at[4 * NQ + j])
        c.start()
        ocopies.append(c)

    def wait(cs):
        for c in cs:
            c.wait()

    A, B_ = list(range(8)), list(range(8, 16))
    jobs = dict(preka=lambda t: pre_k(t)[:1], prekb=lambda t: pre_k(t)[1:], mk=mxu_k, mp=mxu_p, prek=pre_k, postk=post_k, postp=post_p, kvm=lambda: kvm(), kh=mxu_kh,
                postkh=post_kh, z=mxu_z, postz=post_z, pra=lambda j: prod(j, A), prb=lambda j: prod(j, B_),
                inv=mxu_inv, postinv=post_inv, q1=q1, v1=v1, q2=q2, v2=v2, q3=q3, v3=v3)
    MXU_JOBS = ('mk', 'mp', 'kvm', 'kh', 'z', 'inv', 'q1', 'q2', 'q3')

    def deps(name, *a):
        i = a[0] if a else None
        return {
            'mk': lambda: [('prek', i)] if i else [('preka', 0), ('prekb', 0)],
            'postk': lambda: [('mk', i)],
            'postp': lambda: [('mp', i)],
            'kvm': lambda: [('postp', k) for k in range(16)],
            'kh': lambda: [('postk', 2 * i), ('postk', 2 * i + 1)],
            'postkh': lambda: [('kh', i)],
            'postz': lambda: [('z', i)],
            'pra': lambda: [('kh', i), ('z', i)],
            'prb': lambda: [('kh', i), ('z', i)],
            'inv': lambda: [('pra', i), ('prb', i)],
            'postinv': lambda: [('inv', i)],
            'v1': lambda: [('q1', i)],
            'q2': lambda: [('v1', i), ('kvm',)],
            'v2': lambda: [('q2', i)],
            'q3': lambda: [('v2', i), ('kvm',)],
            'v3': lambda: [('q3', i)],
        }.get(name, lambda: [])()

    table = SCHEDULE
    done = {}
    for si, entry in enumerate(table):
        for job in entry['jobs']:
            for d in deps(*job):
                assert d in done and done[d] < si, (si, job, d)
        for job in entry['jobs']:
            done[job] = si
    waits = dict(x0=cps_x[0], x1=cps_x[1], x2=cps_x[2], x3=cps_x[3],
                 wa=[cps_w[4], cps_w[8], cps_w[5], cps_w[9]], wb=[cps_w[6], cps_w[10], cps_w[7], cps_w[11]],
                 c=[cp_c], u=cps_u, wq=cps_w[:4], wo=cps_wo + [cp_dsk], p0=cps_p0, p1=cps_p1)
    for si, entry in enumerate(table):
        for w in entry.get('wait', ()):
            wait(waits[w])
        mj = [jobs[j[0]](*j[1:]) for j in entry['jobs'] if j[0] in MXU_JOBS]
        vj = [jobs[j[0]](*j[1:]) for j in entry['jobs'] if j[0] not in MXU_JOBS]
        slot('s%d' % si, mj, vj)
        for j in entry['jobs']:
            if j[0] == 'v3':
                out_b(j[1])
            if j[0] == 'postinv':
                out_a(j[1])
    wait(ocopies)


@jax.jit
def pallas_concat_heads__ssm_conv_s4__linear_attn_block__prompt_kernel(
    A_u: jax.Array,
    A_A_re: jax.Array,
    A_A_im: jax.Array,
    A_B_re: jax.Array,
    A_B_im: jax.Array,
    A_C_re: jax.Array,
    A_C_im: jax.Array,
    A_log_dt: jax.Array,
    A_Dskip: jax.Array,
    B_x: jax.Array,
    B_wqkv: jax.Array,
    B_wo: jax.Array,
):
    keys, ctab = _constants()
    any_spec = pl.BlockSpec(memory_space=pl.ANY)
    vm = pl.BlockSpec(memory_space=pltpu.VMEM)
    V = pltpu.VMEM

    out = pl.pallas_call(
        functools.partial(_kernel, keys),
        out_shape=jax.ShapeDtypeStruct((L, 2 * D), BF16),
        in_specs=[pl.BlockSpec(memory_space=pltpu.SMEM)] + [any_spec] * 13,
        out_specs=any_spec,
        scratch_shapes=[
            V((4, L, 128), BF16),
            V((4, L, 128), BF16),
            V((12, D, 128), BF16),
            V((4, D, 128), BF16),
            V(ctab.shape, BF16),
            V((6, D, 128), BF16),
            V((D,), BF16),
            V((D,), BF16),
            V((D, 128), F32),
            V((GPI, 2, 2, GROWS // 2, 128), U32),
            V((GPI, 2, 2, 64, 128), U32),
            [V((GPI, 2, 2, GROWS, 128), F32)] * 2,
            V((6, D // 2, 128), U32),
            [V((2, 4, PR_, 128), F32)] * 4,
            V((4, L // 2, 128), U32),
            V((4, L // 2, 128), U32),
            V((4, 4, 8, 8, 128), F32),
            V((4, 64, 128), U32),
            V((4, D // 2, 128), U32),
            V((NCH, ND, C, 128), F32),
            V((NCH, ND, C, 128), F32),
            V((5, ND, 2 * C, 128), F32),
            V((NCH, ND, 2 * C, 128), F32),
            V((NCH, ND, C, 128), U32),
            V((NCH, 2, C, 128), F32),
            [V((4, 4, QR, 128), F32)] * 4,
            V((NQ, 4, QR // 2, 128), U32),
            V((NQ, 4, QR, 128), F32),
            V((NQ, 4, QR // 2, 128), U32),
            [V((4, 4, QR, 128), F32)] * 4,
            V((4, L, 128), BF16),
            V((4, L, 128), BF16),
            pltpu.SemaphoreType.DMA((51,)),
            pltpu.SemaphoreType.DMA((4 * NQ + 4,)),
        ],
        compiler_params=pltpu.CompilerParams(vmem_limit_bytes=120 * 1024 * 1024),
    )(
        jnp.zeros((1,), jnp.int32),
        A_u.reshape(L, D), A_A_re, A_A_im, A_B_re, A_B_im, A_C_re, A_C_im,
        A_log_dt, A_Dskip,
        B_x.reshape(L, D), B_wqkv, B_wo, jnp.asarray(ctab),
    )
    return out.reshape(1, L, 2 * D)
```

```python
import functools

import numpy as np
import jax
import jax.numpy as jnp
from jax import lax
import jax.experimental.pallas as pl
import jax.experimental.pallas.tpu as pltpu

L = 2048
D = 512
NS = 128
C = 128
NCH = L // C
H = 32
DH = D // H
ND = D // 128

F32 = jnp.float32
BF16 = jnp.bfloat16
U32 = jnp.uint32


PAIRS = [(0, 4), (1, 5), (2, 6), (3, 7), (256, 512), (258, 516), (260, 768), (262, 772),
         (1024, 2048), (1280, 512), (1536, 1024), (1792, None)]
NP_ = len(PAIRS)
GROWS = 8 * NP_
NB = 32


def _lane(a_lo, b, slot):
    return 4 * ((b + 1 + a_lo) % NB) + slot


@functools.lru_cache(maxsize=None)
def _constants():
    bf = jnp.bfloat16
    rl = np.arange(L).astype(np.float32).astype(bf).astype(np.int64)
    kperm = np.concatenate([np.arange(0, C, 2), np.arange(1, C, 2)])

    def w(j):
        return np.exp(-1j * np.pi * (2 * kperm + 1) * j / 256.0)

    def main_tiles(al):
        return [0, 3] if al < 2 else [1] if al < 4 else [4] if al < 8 else [2]

    pairs = {}
    for al in range(NCH):
        for j in range(C):
            v = int(rl[C * al + j])
            found = None
            for tl in main_tiles(al) + [5]:
                a_lo, mu = tl // 3, tl % 3
                for slot in range(4):
                    e = PAIRS[4 * mu + slot][a_lo]
                    if e is not None and v >= e and (v - e) % 8 == 0 and (v - e) // 8 < NB:
                        found = (tl, _lane(a_lo, (v - e) // 8, slot))
                        break
                if found:
                    break
            m = pairs.setdefault((al, found[0]), np.zeros((C, C), np.complex128))
            m[:, found[1]] += w(j)
    keys = sorted(pairs.keys())
    fsel = np.stack([np.concatenate([pairs[k].real, pairs[k].imag], 0) for k in keys])
    ff = np.stack([w(j) for j in range(C)], 1)
    ffwd = np.concatenate([ff.real, ff.imag], 0)
    tau = np.arange(C)
    ang = 2 * np.pi * (kperm[None, :] + 0.5) * (C + tau[:, None]) / 256.0
    fre, fim = np.cos(ang) * (2.0 / 256.0), -np.sin(ang) * (2.0 / 256.0)
    finv = np.zeros((2, 128, 128))
    for kb in range(16):
        h, o = kb // 8, 16 * (kb % 8)
        finv[h, :, o:o + 8] = fre[:, 8 * kb:8 * kb + 8]
        finv[h, :, o + 8:o + 16] = fim[:, 8 * kb:8 * kb + 8]
    hid = np.arange(128) // DH
    bmask = (hid[:, None] == hid[None, :]).astype(np.float32)
    tab = np.concatenate([fsel.reshape(-1, 128), ffwd, finv.reshape(-1, 128), bmask], 0)
    return tuple(keys), tab.astype(bf)


def _cmul(ar, ai, br, bi):
    return ar * br - ai * bi, ar * bi + ai * br


def _nt(a, b):
    return lax.dot_general(a, b, (((1,), (1,)), ((), ())), preferred_element_type=F32)


def _tn(a, b):
    return lax.dot_general(a, b, (((0,), (0,)), ((), ())), preferred_element_type=F32)


def _nn(a, b):
    return jnp.dot(a, b, preferred_element_type=F32)


def _phi(t):
    return jnp.where(t > 0, t + 1.0, jnp.exp(t)) + 1e-6


def _ld(ref_u32, *idx):
    *lead, (r0, n) = idx
    return pltpu.bitcast(ref_u32[(*lead, slice(r0 // 2, (r0 + n) // 2), slice(None))], BF16)


def _pk(x):
    return pltpu.bitcast(x.astype(BF16), U32)


def _sincos(x):
    n = jnp.round(x * 0.6366197723675814)
    r = x - n * 1.5703125
    r = r - n * 4.837512969970703e-04
    r = r - n * 7.549789954891882e-08
    r2 = r * r
    sp = r + r * r2 * (-1.6666654611e-01 + r2 * (8.3321608736e-03 + r2 * (-1.9515295891e-04)))
    cp = 1.0 - 0.5 * r2 + r2 * r2 * (4.166664568298827e-02 + r2 * (-1.388731625493765e-03 + r2 * 2.443315711809948e-05))
    q = n.astype(jnp.int32)
    swap = (q & 1) == 1
    sn = jnp.where(swap, cp, sp)
    cs = jnp.where(swap, sp, cp)
    sn = jnp.where((q & 2) == 2, -sn, sn)
    cs = jnp.where(((q + 1) & 2) == 2, -cs, cs)
    return sn, cs


def _rev4(x):
    sub = lax.broadcasted_iota(jnp.int32, x.shape, 0)
    for bit in (2, 1):
        up = pltpu.roll(x, 8 - bit, 0)
        dn = pltpu.roll(x, bit, 0)
        x = jnp.where((sub & bit) == 0, up, dn)
    return x


GPI = 8
RB = 8 * GPI
NKI = D // RB
PR_ = 512
QR = 256
NQ = L // QR


MB = 1.2

SCHEDULE = [
    dict(wait=['p0'], jobs=[('preka', 0)]),
    dict(wait=['x0', 'wa'], jobs=[('mp', 0), ('mp', 1), ('prekb', 0)]),
    dict(wait=['wb', 'p1'], jobs=[('mk', 0), ('mp', 2), ('mp', 3), ('postp', 0), ('postp', 1), ('prek', 1)]),
    dict(wait=['x1'], jobs=[('mk', 1), ('mp', 4), ('mp', 5), ('postk', 0), ('postp', 2), ('postp', 3), ('prek', 2)]),
    dict(jobs=[('mk', 2), ('mp', 6), ('mp', 7), ('postk', 1), ('postp', 4), ('postp', 5), ('prek', 3)]),
    dict(wait=['x2', 'c', 'u'], jobs=[('mk', 3), ('mp', 8), ('mp', 9), ('za', 0), ('postk', 2), ('postp', 6), ('postp', 7), ('prek', 4)]),
    dict(jobs=[('mk', 4), ('mp', 10), ('mp', 11), ('zb', 0), ('postk', 3), ('postp', 8), ('postp', 9), ('prek', 5)]),
    dict(wait=['x3'], jobs=[('mk', 5), ('mp', 12), ('mp', 13), ('kha', 0), ('postk', 4), ('postp', 10), ('postp', 11), ('prek', 6)]),
    dict(jobs=[('mk', 6), ('mp', 14), ('mp', 15), ('khb', 0), ('postk', 5), ('postp', 12), ('postp', 13), ('prek', 7)]),
    dict(jobs=[('mk', 7), ('kha', 1), ('khb', 1), ('za', 1), ('zb', 1), ('postk', 6), ('postp', 14), ('postp', 15), ('pra', 0)]),
    dict(wait=['wq', 'wo'], jobs=[('kvm',), ('kha', 2), ('khb', 2), ('q1', 0), ('postk', 7)]),
    dict(jobs=[('kha', 3), ('khb', 3), ('za', 2), ('zb', 2), ('q1', 1), ('v1', 0), ('prb', 0)]),
    dict(jobs=[('za', 3), ('zb', 3), ('q2', 0), ('q1', 2), ('q1', 3), ('v1', 1), ('pra', 1)]),
    dict(jobs=[('inv', 0), ('q1', 4), ('q2', 1), ('q1', 5), ('v1', 2), ('v1', 3), ('v2', 0), ('prb', 1)]),
    dict(jobs=[('q2', 2), ('q2', 3), ('q3', 0), ('q1', 6), ('v1', 4), ('v1', 5), ('v2', 1), ('postinv', 0), ('pra', 2)]),
    dict(jobs=[('inv', 1), ('q2', 4), ('q2', 5), ('q3', 1), ('q1', 7), ('v1', 6), ('v2', 2), ('v2', 3), ('v3', 0), ('prb', 2)]),
    dict(jobs=[('q2', 6), ('q3', 2), ('q3', 3), ('v1', 7), ('v2', 4), ('v2', 5), ('v3', 1), ('postinv', 1), ('pra', 3)]),
    dict(jobs=[('inv', 2), ('q2', 7), ('q3', 4), ('q3', 5), ('v2', 6), ('v3', 2), ('v3', 3), ('prb', 3)]),
    dict(jobs=[('inv', 3), ('q3', 6), ('v2', 7), ('v3', 4), ('v3', 5), ('postinv', 2)]),
    dict(jobs=[('q3', 7), ('v3', 6), ('postinv', 3)]),
    dict(jobs=[('v3', 7)]),
]


def _kernel(keys,
            z_ref, u_hbm, are_hbm, aim_hbm, bre_hbm, bim_hbm, cre_hbm, cim_hbm, ldt_hbm, dsk_hbm,
            x_hbm, wqkv_hbm, wo_hbm, ctab_hbm,
            out_hbm,
            u_v, x_v, w_v, wo_v, ctab_v, par_v, ldt_v, dsk_v,
            dtc_v, g_v, h_v, rk_v, kt_v, rp_v, pk_v, v_v, zp_v, zrow_v, m_v,
            kp_v, ki_v, kx_v, zr_v, yh_v, ri_v,
            rq_v, pz_v, rd_v, o_v, ro_v,
            oa_v, ob_v, sems, osems):
    npair = len(keys)
    z = z_ref[0]

    def slot(name, mjobs, vjobs):
        seq = []
        mp = [p for j in mjobs for p in j]
        mt = sum(c for c, _ in mp) or 1
        acc = 0
        for c, f in mp:
            seq.append((MB * acc / mt, 0, f))
            acc += c
        for j in vjobs:
            vt = sum(c for c, _ in j) or 1
            acc = 0
            for c, f in j:
                seq.append((acc / vt + 1e-6, 1, f))
                acc += c
        seq.sort(key=lambda e: (e[0], e[1]))
        with jax.named_scope(name):
            @pl.when(z == 0)
            def _():
                for _, _, f in seq:
                    f()

    def cp(src, dst, k):
        return pltpu.make_async_copy(src, dst, sems.at[k])

    cps_w = [cp(wqkv_hbm.at[:, pl.ds(128 * n, 128)], w_v.at[n], n) for n in range(12)]
    cps_x = [[cp(x_hbm.at[pl.ds(PR_ * rb, PR_), pl.ds(128 * kk, 128)], x_v.at[kk, pl.ds(PR_ * rb, PR_), :],
                 12 + 4 * rb + kk) for kk in range(4)] for rb in range(4)]
    cps_u = [cp(u_hbm.at[:, pl.ds(128 * j, 128)], u_v.at[j], 28 + j) for j in range(4)]
    cps_wo = [cp(wo_hbm.at[:, pl.ds(128 * n, 128)], wo_v.at[n], 32 + n) for n in range(4)]
    cp_c = cp(ctab_hbm, ctab_v, 36)
    par_hbm = (are_hbm, aim_hbm, bre_hbm, bim_hbm, cre_hbm, cim_hbm)
    cps_p0 = [cp(h.at[pl.ds(0, RB), :], par_v.at[i, pl.ds(0, RB), :], 37 + i) for i, h in enumerate(par_hbm)]
    cps_p1 = [cp(h.at[pl.ds(RB, D - RB), :], par_v.at[i, pl.ds(RB, D - RB), :], 43 + i) for i, h in enumerate(par_hbm)]
    cp_ldt = cp(ldt_hbm, ldt_v, 49)
    cp_dsk = cp(dsk_hbm, dsk_v, 50)
    order = ([cp_ldt] + cps_p0 + cps_x[0] + [cps_w[4], cps_w[8], cps_w[5], cps_w[9]] + cps_p1
             + [cps_w[6], cps_w[10], cps_w[7], cps_w[11]]
             + cps_x[1] + cps_x[2] + [cp_c] + cps_u + cps_x[3] + cps_w[:4] + cps_wo + [cp_dsk])
    for c in order:
        c.start()
    are_ref, aim_ref, bre_ref, bim_ref, cre_ref, cim_ref = (par_v.at[i] for i in range(6))

    xu, wu, uu, wou, cu = (r.bitcast(U32) for r in (x_v, w_v, u_v, wo_v, ctab_v))
    off_ffwd = npair * 256
    off_finv = off_ffwd + 256
    off_bm = off_finv + 256

    cp_ldt.wait()
    dt_row = jnp.exp(ldt_v[...].astype(F32).reshape(1, D)).astype(BF16).astype(F32)
    dtc_v[...] = jnp.transpose(jnp.broadcast_to(dt_row, (128, D)))

    def pre_k(t):
        def gen(q):
            rows = slice(RB * t + 8 * q, RB * t + 8 * q + 8)
            dt = dtc_v[rows, :]
            lre = dt * are_ref[rows, :].astype(F32)
            lim = dt * aim_ref[rows, :].astype(F32)
            mag = jnp.exp(lre)
            sn, cs = _sincos(lim)
            p1 = (mag * cs, mag * sn)
            dbr = dt * bre_ref[rows, :].astype(F32)
            dbi = dt * bim_ref[rows, :].astype(F32)
            c0 = _cmul(cre_ref[rows, :].astype(F32), cim_ref[rows, :].astype(F32), dbr, dbi)
            yield
            pw = {1: p1}
            pw[2] = _cmul(*p1, *p1)
            yield
            pw[3] = _cmul(*pw[2], *p1)
            pw[4] = _cmul(*pw[2], *pw[2])
            yield
            pw[5] = _cmul(*pw[4], *p1)
            pw[6] = _cmul(*pw[4], *pw[2])
            pw[7] = _cmul(*pw[4], *pw[3])
            p8 = _cmul(*pw[4], *pw[4])
            yield
            low = lax.broadcasted_iota(jnp.int32, (8, 128), 0) < 4

            def emit(dst, part, idx, pend, a, b):
                pend.append((jnp.where(low, a, pltpu.roll(b, 4, 0)), jnp.where(low, pltpu.roll(a, 4, 0), b)))
                if len(pend) == 2:
                    r0 = 8 * (idx // 2)
                    dst[q, 0, part, r0:r0 + 8, :] = _pk(jnp.concatenate([pend[0][0], pend[1][0]], axis=0))
                    dst[q, 1, part, r0:r0 + 8, :] = _pk(jnp.concatenate([pend[0][1], pend[1][1]], axis=0))
                    pend.clear()

            p16 = _cmul(*p8, *p8)
            h8 = (_rev4(p8[0]), -_rev4(p8[1]))
            h16 = _cmul(*h8, *h8)
            yield
            p32 = _cmul(*p16, *p16)
            yield
            p64 = _cmul(*p32, *p32)
            yield
            p128 = _cmul(*p64, *p64)
            yield
            p256 = _cmul(*p128, *p128)
            yield
            zero = jnp.zeros((8, 128), F32)
            gt = {0: c0, None: (zero, zero)}

            def grow(e):
                if e not in gt:
                    if e % 256 == 0:
                        gt[e] = _cmul(*grow(e - 256), *p256)
                    else:
                        gt[e] = _cmul(*grow(256 * (e // 256)), *pw[e % 256])
                return gt[e]

            h0 = (jnp.ones((8, 128), F32), jnp.zeros((8, 128), F32))
            hr, hi_, gr, gi = [], [], [], []
            for be in range(NB // 2):
                h1 = h8 if be == 0 else _cmul(*h0, *h8)
                hn = None
                if be + 1 < NB // 2:
                    hn = h16 if be == 0 else _cmul(*h0, *h16)
                emit(h_v, 0, be, hr, h0[0], h1[0])
                emit(h_v, 1, be, hi_, h0[1], h1[1])
                h0 = hn
                if be < NP_:
                    a, b = grow(PAIRS[be][0]), grow(PAIRS[be][1])
                    emit(g_v, 0, be, gr, a[0], b[0])
                    emit(g_v, 1, be, gi, a[1], b[1])
                yield

        def piece(q2):
            gens = [gen(2 * q2), gen(2 * q2 + 1)]
            while gens:
                for g in list(gens):
                    try:
                        next(g)
                    except StopIteration:
                        gens.remove(g)
        return [(1600, functools.partial(piece, q2)) for q2 in range(GPI // 2)]

    def mxu_k(t):
        def piece(q2):
            for q in (2 * q2, 2 * q2 + 1):
                for par in range(2):
                    for hf in range(2):
                        rk_v[t % 2][q, par, hf] = _nt(pltpu.bitcast(g_v[q, par, hf], BF16),
                                                      pltpu.bitcast(h_v[q, par, hf], BF16))
        return [(192, functools.partial(piece, q2)) for q2 in range(GPI // 2)]

    def post_k(t):
        def piece(q2):
            lane = lax.broadcasted_iota(jnp.int32, (8, 128), 1)
            low = lax.broadcasted_iota(jnp.int32, (8, 128), 0) < 4
            r = rk_v[t % 2]
            tiles = [[] for _ in range(6)]
            for q in (2 * q2, 2 * q2 + 1):
                acc = [[jnp.zeros((8, 128), F32)] * 3 for _ in range(2)]
                for par in range(2):
                    for pp in range(NP_):
                        mu, sl = pp // 4, pp % 4
                        o = r[q, par, 0, 8 * pp:8 * pp + 8, :] + r[q, par, 1, 8 * pp:8 * pp + 8, :]
                        rolled = pltpu.roll(o, sl + 1, 1, stride=1, stride_axis=0)
                        acc[par][mu] = jnp.where(lane % 4 == sl, rolled, acc[par][mu])
                for mu in range(3):
                    x, y = acc[0][mu], acc[1][mu]
                    tiles[mu].append(jnp.where(low, x, pltpu.roll(y, 4, 0)))
                    tiles[3 + mu].append(jnp.where(low, pltpu.roll(x, 4, 0), y))
            r0 = (RB * t + 16 * q2) // 2
            for tl in range(6):
                kt_v[tl, r0:r0 + 8, :] = _pk(jnp.concatenate(tiles[tl], axis=0))
        return [(190, functools.partial(piece, q2)) for q2 in range(GPI // 2)]

    def proj(r0, nr, n, dst):
        for kk in range(4):
            dst[kk] = _nn(_ld(xu, kk, (r0, nr)), _ld(wu, n, (128 * kk, 128)))

    def mxu_p(i):
        rb, p = i // 4, i % 4
        return [(512, functools.partial(proj, PR_ * rb, PR_, 4 + p, rp_v[i % 4].at[0])),
                (512, functools.partial(proj, PR_ * rb, PR_, 8 + p, rp_v[i % 4].at[1]))]

    def post_p(i):
        def piece(c):
            rb, p = i // 4, i % 4
            r = rp_v[i % 4]
            zacc = None
            for r0 in range(64 * c, 64 * c + 64, 16):
                rs = slice(r0, r0 + 16)
                k = _phi((r[0, 0, rs, :] + r[0, 1, rs, :]) + (r[0, 2, rs, :] + r[0, 3, rs, :]))
                kb = k.astype(BF16)
                o8 = (PR_ * rb + r0) // 2
                pk_v[p, o8:o8 + 8, :] = pltpu.bitcast(kb, U32)
                zz = k[:8] + k[8:]
                zacc = zz if zacc is None else zacc + zz
                v_v[p, o8:o8 + 8, :] = _pk((r[1, 0, rs, :] + r[1, 1, rs, :]) + (r[1, 2, rs, :] + r[1, 3, rs, :]))
            zp_v[rb, p, c] = zacc
        return [(150, functools.partial(piece, c)) for c in range(PR_ // 64)]

    def kvm_piece(blk):
        bmask = _ld(cu, (off_bm, 128))
        if True:
            kv = _tn(_ld(pk_v, blk, (0, L)), _ld(v_v, blk, (0, L))) * bmask.astype(F32)
            kvb = kv.astype(BF16)
            for n in range(4):
                m_v[n, 64 * blk:64 * blk + 64, :] = _pk(_nn(kvb, _ld(wou, n, (128 * blk, 128))))
            zs = sum(zp_v[rb, blk, c] for rb in range(4) for c in range(8))
            zrow = jnp.sum(zs, axis=0, keepdims=True)
            zcol = jnp.transpose(jnp.broadcast_to(zrow, (128, 128)))
            zrow_v[blk] = _pk(zcol * bmask.astype(F32))

    def kvm():
        return [(650, functools.partial(kvm_piece, blk)) for blk in range(4)]

    main_pair = {}
    extra_pair = {}
    for pi, (al, tl) in enumerate(keys):
        if al in main_pair:
            extra_pair[al] = (pi, tl)
        else:
            main_pair[al] = (pi, tl)
    xidx = {al: i for i, al in enumerate(sorted(extra_pair))}

    def mxu_kh(j):
        def piece(c):
            for al in range(4 * c, 4 * c + 4):
                pi, tl = main_pair[al]
                r = _nt(_ld(cu, (256 * pi, 256)), _ld(kt_v, tl, (128 * j, 128)))
                kp_v[al, j] = r[:C]
                ki_v[al, j] = r[C:]
                if al in extra_pair:
                    pi, tl = extra_pair[al]
                    kx_v[xidx[al], j] = _nt(_ld(cu, (256 * pi, 256)), _ld(kt_v, tl, (128 * j, 128)))
        return [(336, functools.partial(piece, c)) for c in range(4)]

    def mxu_z(j):
        def piece(c):
            for a in range(4 * c, 4 * c + 4):
                zr_v[a, j] = _nn(_ld(cu, (off_ffwd, 256)), _ld(uu, j, (C * a, C)))
        return [(256, functools.partial(piece, c)) for c in range(4)]

    def prod_blk(j, kb, a0):
        rs = slice(8 * kb, 8 * kb + 8)
        ri = slice(C + 8 * kb, C + 8 * kb + 8)
        acc = [[None] * 3 for _ in range(4)]
        uc = {}
        zc = {}

        def zraw(a):
            if a not in zc:
                zc[a] = (zr_v[a, j, rs, :], zr_v[a, j, ri, :])
            return zc[a]

        for al in range(a0 + 4):
            kr, ki = kp_v[al, j, rs, :], ki_v[al, j, rs, :]
            if al in extra_pair:
                kr = kr + kx_v[xidx[al], j, rs, :]
                ki = ki + kx_v[xidx[al], j, ri, :]
            kk = (kr, ki - kr, kr + ki)
            for o in range(3, -1, -1):
                ap = a0 + o - al
                if ap < 0:
                    continue
                if ap not in uc:
                    zr, zi = zraw(ap)
                    if ap == 0:
                        ar, ai = (zi, -zr) if kb < 8 else (-zi, zr)
                    else:
                        pr, pi = zraw(ap - 1)
                        ar, ai = (pr + zi, pi - zr) if kb < 8 else (pr - zi, pi + zr)
                    uc[ap] = (ar + ai, ar, ai)
                ux = uc[ap]
                for w in range(3):
                    tt = kk[w] * ux[w]
                    acc[o][w] = tt if acc[o][w] is None else acc[o][w] + tt
        return [(acc[o][0] - acc[o][2], acc[o][0] + acc[o][1]) for o in range(4)]

    def prod(j, kbs):
        def piece(kb, a0):
            r = prod_blk(j, kb, a0)
            for o in range(4):
                yh_v[a0 + o, j, 8 * kb:8 * kb + 8, :] = _pk(jnp.concatenate([r[o][0], r[o][1]], axis=0))
        return [(6 * (4 * a0 + 10) + 5 * (a0 + 4) + 15, functools.partial(piece, kb, a0)) for kb in kbs for a0 in range(0, NCH, 4)]

    def mxu_inv(j):
        def piece(c):
            for a in range(4 * c, 4 * c + 4):
                for hf in range(2):
                    ri_v[j % 2, a, hf] = _nn(_ld(cu, (off_finv + 128 * hf, 128)), _ld(yh_v, a, j, (128 * hf, 128)))
        return [(256, functools.partial(piece, c)) for c in range(4)]

    def post_inv(j):
        def piece(c):
            dsk = dsk_v[...].astype(F32).reshape(1, D)[:, 128 * j:128 * j + 128]
            for a in (c,):
                for r0 in range(0, C, 16):
                    rs = slice(r0, r0 + 16)
                    y = ri_v[j % 2, a, 0, rs, :] + ri_v[j % 2, a, 1, rs, :]
                    ud = _ld(uu, j, (C * a + r0, 16)).astype(F32) * dsk
                    oa_v[j, C * a + r0:C * a + r0 + 16, :] = (y + ud).astype(BF16)
        return [(90, functools.partial(piece, c)) for c in range(NCH)]

    def q1(i):
        return [(256, functools.partial(proj, QR * i, QR, n, rq_v[i % 4].at[n])) for n in range(4)]

    def v1(i):
        def piece(n, c):
            r = rq_v[i % 4]
            if True:
                for r0 in range(64 * c, 64 * c + 64, 16):
                    rs = slice(r0, r0 + 16)
                    pq = _phi((r[n, 0, rs, :] + r[n, 1, rs, :]) + (r[n, 2, rs, :] + r[n, 3, rs, :]))
                    pz_v[i, n, r0 // 2:r0 // 2 + 8, :] = _pk(pq)
        return [(100, functools.partial(piece, n, c)) for n in range(4) for c in range(QR // 64)]

    def q2(i):
        def piece():
            for n in range(4):
                rd_v[i, n] = _nn(pltpu.bitcast(pz_v[i, n], BF16), pltpu.bitcast(zrow_v[n], BF16))
        return [(256, piece)]

    def v2(i):
        def piece(n, c):
            if True:
                for r0 in range(64 * c, 64 * c + 64, 16):
                    rs = slice(r0, r0 + 16)
                    o_v[i, n, r0 // 2:r0 // 2 + 8, :] = _pk(_ld(pz_v, i, n, (r0, 16)).astype(F32) * pl.reciprocal(rd_v[i, n, rs, :] + 1e-6, approx=True))
        return [(75, functools.partial(piece, n, c)) for n in range(4) for c in range(QR // 64)]

    def q3(i):
        def piece(n):
            if True:
                for kk in range(4):
                    ro_v[i % 4][n, kk] = _nn(pltpu.bitcast(o_v[i, kk], BF16), _ld(m_v, n, (128 * kk, 128)))
        return [(256, functools.partial(piece, n)) for n in range(4)]

    def v3(i):
        def piece(n, c):
            r = ro_v[i % 4]
            if True:
                for r0 in range(64 * c, 64 * c + 64, 16):
                    rs = slice(r0, r0 + 16)
                    ob_v[n, QR * i + r0:QR * i + r0 + 16, :] = (
                        (r[n, 0, rs, :] + r[n, 1, rs, :]) + (r[n, 2, rs, :] + r[n, 3, rs, :])).astype(BF16)
        return [(40, functools.partial(piece, n, c)) for n in range(4) for c in range(QR // 64)]

    ocopies = []

    def out_b(i):
        for n in range(4):
            c = pltpu.make_async_copy(ob_v.at[n, pl.ds(QR * i, QR), :],
                                      out_hbm.at[pl.ds(QR * i, QR), pl.ds(D + 128 * n, 128)], osems.at[4 * i + n])
            c.start()
            ocopies.append(c)

    def out_a(j):
        c = pltpu.make_async_copy(oa_v.at[j], out_hbm.at[:, pl.ds(128 * j, 128)], osems.at[4 * NQ + j])
        c.start()
        ocopies.append(c)

    def wait(cs):
        for c in cs:
            c.wait()

    A, B_ = list(range(8)), list(range(8, 16))
    jobs = dict(preka=lambda t: pre_k(t)[:1], prekb=lambda t: pre_k(t)[1:], mk=mxu_k, mp=mxu_p, prek=pre_k, postk=post_k, postp=post_p, kvm=lambda: kvm(), kha=lambda j: mxu_kh(j)[:2], khb=lambda j: mxu_kh(j)[2:],
                za=lambda j: mxu_z(j)[:2], zb=lambda j: mxu_z(j)[2:], pra=lambda j: prod(j, A), prb=lambda j: prod(j, B_),
                inv=mxu_inv, postinv=post_inv, q1=q1, v1=v1, q2=q2, v2=v2, q3=q3, v3=v3)
    MXU_JOBS = ('mk', 'mp', 'kvm', 'kha', 'khb', 'za', 'zb', 'inv', 'q1', 'q2', 'q3')

    def deps(name, *a):
        i = a[0] if a else None

        def prev(n, k):
            return [(n, k)] if k >= 0 else []
        return {
            'mk': lambda: ([('prek', i)] if i else [('preka', 0), ('prekb', 0)]) + prev('postk', i - 2),
            'mp': lambda: prev('postp', i - 4),
            'postk': lambda: [('mk', i)],
            'postp': lambda: [('mp', i)],
            'kvm': lambda: [('postp', k) for k in range(16)],
            'kha': lambda: [('postk', 2 * i), ('postk', 2 * i + 1)],
            'khb': lambda: [('postk', 2 * i), ('postk', 2 * i + 1)],
            'pra': lambda: [('kha', i), ('khb', i), ('za', i), ('zb', i)],
            'prb': lambda: [('kha', i), ('khb', i), ('za', i), ('zb', i)],
            'inv': lambda: [('pra', i), ('prb', i)] + prev('postinv', i - 2),
            'postinv': lambda: [('inv', i)],
            'q1': lambda: prev('v1', i - 4),
            'v1': lambda: [('q1', i)],
            'q2': lambda: [('v1', i), ('kvm',)],
            'v2': lambda: [('q2', i)],
            'q3': lambda: [('v2', i), ('kvm',)] + prev('v3', i - 4),
            'v3': lambda: [('q3', i)],
        }.get(name, lambda: [])()

    table = SCHEDULE
    done = {}
    for si, entry in enumerate(table):
        for job in entry['jobs']:
            for d in deps(*job):
                assert d in done and done[d] < si, (si, job, d)
        for job in entry['jobs']:
            done[job] = si
        for job in entry['jobs']:
            if job[0] == 'prek':
                assert ('mk', job[1] - 1) in done, job
    waits = dict(x0=cps_x[0], x1=cps_x[1], x2=cps_x[2], x3=cps_x[3],
                 wa=[cps_w[4], cps_w[8], cps_w[5], cps_w[9]], wb=[cps_w[6], cps_w[10], cps_w[7], cps_w[11]],
                 c=[cp_c], u=cps_u, wq=cps_w[:4], wo=cps_wo + [cp_dsk], p0=cps_p0, p1=cps_p1)
    for si, entry in enumerate(table):
        for w in entry.get('wait', ()):
            wait(waits[w])
        mj = [jobs[j[0]](*j[1:]) for j in entry['jobs'] if j[0] in MXU_JOBS]
        vj = [jobs[j[0]](*j[1:]) for j in entry['jobs'] if j[0] not in MXU_JOBS]
        slot('s%d' % si, mj, vj)
        for j in entry['jobs']:
            if j[0] == 'v3':
                out_b(j[1])
            if j[0] == 'postinv':
                out_a(j[1])
    wait(ocopies)


@jax.jit
def pallas_concat_heads__ssm_conv_s4__linear_attn_block__prompt_kernel(
    A_u: jax.Array,
    A_A_re: jax.Array,
    A_A_im: jax.Array,
    A_B_re: jax.Array,
    A_B_im: jax.Array,
    A_C_re: jax.Array,
    A_C_im: jax.Array,
    A_log_dt: jax.Array,
    A_Dskip: jax.Array,
    B_x: jax.Array,
    B_wqkv: jax.Array,
    B_wo: jax.Array,
):
    keys, ctab = _constants()
    any_spec = pl.BlockSpec(memory_space=pl.ANY)
    V = pltpu.VMEM

    out = pl.pallas_call(
        functools.partial(_kernel, keys),
        out_shape=jax.ShapeDtypeStruct((L, 2 * D), BF16),
        in_specs=[pl.BlockSpec(memory_space=pltpu.SMEM)] + [any_spec] * 13,
        out_specs=any_spec,
        scratch_shapes=[
            V((4, L, 128), BF16),
            V((4, L, 128), BF16),
            V((12, D, 128), BF16),
            V((4, D, 128), BF16),
            V(ctab.shape, BF16),
            V((6, D, 128), BF16),
            V((D,), BF16),
            V((D,), BF16),
            V((D, 128), F32),
            V((GPI, 2, 2, GROWS // 2, 128), U32),
            V((GPI, 2, 2, 64, 128), U32),
            [V((GPI, 2, 2, GROWS, 128), F32)] * 2,
            V((6, D // 2, 128), U32),
            [V((2, 4, PR_, 128), F32)] * 4,
            V((4, L // 2, 128), U32),
            V((4, L // 2, 128), U32),
            V((4, 4, 8, 8, 128), F32),
            V((4, 64, 128), U32),
            V((4, D // 2, 128), U32),
            V((NCH, ND, C, 128), F32),
            V((NCH, ND, C, 128), F32),
            V((5, ND, 2 * C, 128), F32),
            V((NCH, ND, 2 * C, 128), F32),
            V((NCH, ND, C, 128), U32),
            V((2, NCH, 2, C, 128), F32),
            [V((4, 4, QR, 128), F32)] * 4,
            V((NQ, 4, QR // 2, 128), U32),
            V((NQ, 4, QR, 128), F32),
            V((NQ, 4, QR // 2, 128), U32),
            [V((4, 4, QR, 128), F32)] * 4,
            V((4, L, 128), BF16),
            V((4, L, 128), BF16),
            pltpu.SemaphoreType.DMA((51,)),
            pltpu.SemaphoreType.DMA((4 * NQ + 4,)),
        ],
        compiler_params=pltpu.CompilerParams(vmem_limit_bytes=120 * 1024 * 1024),
    )(
        jnp.zeros((1,), jnp.int32),
        A_u.reshape(L, D), A_A_re, A_A_im, A_B_re, A_B_im, A_C_re, A_C_im,
        A_log_dt, A_Dskip,
        B_x.reshape(L, D), B_wqkv, B_wo, jnp.asarray(ctab),
    )
    return out.reshape(1, L, 2 * D)
```
